```python
import jax
import jax.numpy as jnp

def _softmax(x, axis=-1):
    return jax.nn.softmax(x, axis=axis)

def _gelu(x):
    return jax.nn.gelu(x, approximate=True)

def _silu(x):
    return jax.nn.silu(x)

def _sigmoid(x):
    return jax.nn.sigmoid(x)

def _layernorm(x, axis=-1, eps=1e-05):
    m = jnp.mean(x, axis=axis, keepdims=True)
    v = jnp.var(x, axis=axis, keepdims=True)
    return (x - m) / jnp.sqrt(v + eps)

def _scatter_add(tgt, idx, src, axis=0):
    return tgt.at[idx].add(src)

def _segment_sum(src, seg, n):
    return jax.ops.segment_sum(src, seg, n)

class _Rng:

    def __init__(self, key):
        self._k = key

    def _next(self):
        self._k, sub = jax.random.split(self._k)
        return sub

    def normal(self, shape):
        return jax.random.normal(self._next(), shape, dtype=jnp.bfloat16)

    def randint(self, lo, hi, shape):
        return jax.random.randint(self._next(), shape, lo, hi, dtype=jnp.int32)

    def uniform(self, shape, lo=0.0, hi=1.0):
        return jax.random.uniform(self._next(), shape, jnp.bfloat16, lo, hi)

    def permutation(self, n):
        return jax.random.permutation(self._next(), n)
kernel_name = 'adaLN_cond__compressed_kv_cla__mixer_s_mlp__prompt'

def setup_inputs():
    _rng = _Rng(jax.random.key(int.from_bytes(__import__("os").urandom(4), "little")))
    _w = lambda a: (lambda t: t.astype(jnp.bfloat16) if jnp.issubdtype(t.dtype, jnp.floating) else t)(jnp.asarray(a))

    def _A_setup():
        B, H, Sq, Sk, D, M = (1, 32, 2048, 2048, 128, 640)
        Dc = 4 * D
        return {'x': _w((lambda *s: _rng.normal(s) * 0.05)(B, Sq, M)), 'c_kv': _w((lambda *s: _rng.normal(s) * 0.05)(B, Sk, Dc)), 'w_q': _w((lambda *s: _rng.normal(s) * 0.05)(M, H, D) * M ** (-0.5)), 'w_uk': _w((lambda *s: _rng.normal(s) * 0.05)(Dc, H, D) * Dc ** (-0.5)), 'w_uv': _w((lambda *s: _rng.normal(s) * 0.05)(Dc, H, D) * Dc ** (-0.5)), 'w_o': _w((lambda *s: _rng.normal(s) * 0.05)(H, D, M) * (H * D) ** (-0.5))}
    _A_in = _A_setup()

    def _B_setup():
        B, S, D, F = (1, 2048, 640, 1728)
        return {'x': _w((lambda *s: _rng.normal(s) * 0.05)(B, S, D)), 'w1': _w((lambda *s: _rng.normal(s) * 0.05)(D, D) * D ** (-0.5)), 'w2': _w((lambda *s: _rng.normal(s) * 0.05)(D, D) * D ** (-0.5)), 'w3': _w((lambda *s: _rng.normal(s) * 0.05)(D, F) * D ** (-0.5)), 'w4': _w((lambda *s: _rng.normal(s) * 0.05)(F, D) * F ** (-0.5))}
    _B_in = _B_setup()
    return {'A_x': _A_in['x'], 'A_c_kv': _A_in['c_kv'], 'A_w_q': _A_in['w_q'], 'A_w_uk': _A_in['w_uk'], 'A_w_uv': _A_in['w_uv'], 'A_w_o': _A_in['w_o'], 'B_x': _B_in['x'], 'B_w1': _B_in['w1'], 'B_w2': _B_in['w2'], 'B_w3': _B_in['w3'], 'B_w4': _B_in['w4'], 'c': _w((lambda *s: _rng.normal(s) * 0.05)(1, 640)), 'w_mod': _w((lambda *s: _rng.normal(s) * 0.05)(640, 6 * 640) * 640 ** (-0.5))}

def reference(A_x, A_c_kv, A_w_q, A_w_uk, A_w_uv, A_w_o, B_x, B_w1, B_w2, B_w3, B_w4, c, w_mod):

    def _A_ref(x, c_kv, w_q, w_uk, w_uv, w_o):
        B, Sq, M = (x.shape[0], x.shape[1], x.shape[2])
        Sk = c_kv.shape[1]
        H, D = (w_q.shape[1], w_q.shape[2])
        q = jnp.einsum('bqm,mhd->bhqd', x, w_q)
        k = jnp.einsum('bkc,chd->bhkd', c_kv, w_uk)
        v = jnp.einsum('bkc,chd->bhkd', c_kv, w_uv)
        scores = jnp.einsum('bhqd,bhkd->bhqk', q, k) * D ** (-0.5)
        off = Sk - Sq
        qi = jnp.arange(Sq)[:, None]
        kj = jnp.arange(Sk)[None, :]
        cmask = kj <= qi + off
        scores = jnp.where(cmask[None, None], scores, -1000000000.0)
        p = _softmax(scores, axis=-1)
        ctx = jnp.einsum('bhqk,bhkd->bhqd', p, v)
        return jnp.einsum('bhqd,hdm->bqm', ctx, w_o)

    def _B_ref(x, w1, w2, w3, w4):
        B, S, D = x.shape
        h = _gelu(_layernorm(x, axis=-1) @ w1)
        c = D // 4
        g0 = jnp.pad(h[:, :, 0 * c:1 * c], ((0, 0), (1, 0), (0, 0)))[:, :S, :]
        g1 = jnp.pad(h[:, :, 1 * c:2 * c], ((0, 0), (0, 1), (0, 0)))[:, 1:, :]
        g2 = jnp.pad(h[:, :, 2 * c:3 * c], ((0, 0), (2, 0), (0, 0)))[:, :S, :]
        g3 = jnp.pad(h[:, :, 3 * c:], ((0, 0), (0, 2), (0, 0)))[:, 2:, :]
        hs = jnp.concatenate([g0, g1, g2, g3], axis=-1) @ w2
        x1 = x + hs
        h2 = _gelu(_layernorm(x1, axis=-1) @ w3) @ w4
        return x1 + h2
    x = A_x
    mod = (_silu(c) @ w_mod).reshape(c.shape[0], 6, 1, -1)
    sa, ca, ga, sb, cb, gb = (mod[:, 0].copy(), mod[:, 1].copy(), mod[:, 2].copy(), mod[:, 3].copy(), mod[:, 4].copy(), mod[:, 5].copy())
    h = _layernorm(x, axis=-1) * (1 + ca) + sa
    x = x + ga * _A_ref(h, A_c_kv, A_w_q, A_w_uk, A_w_uv, A_w_o)
    h = _layernorm(x, axis=-1) * (1 + cb) + sb
    x = x + gb * _B_ref(h, B_w1, B_w2, B_w3, B_w4)
    return x
```

```python
import math

import jax
import jax.numpy as jnp
import jax.experimental.pallas as pl
import jax.experimental.pallas.tpu as pltpu

F32 = jnp.float32
BF16 = jnp.bfloat16
U32 = jnp.uint32
NT = (((1,), (1,)), ((), ()))
T = 128
EPS = 1e-5
LOG2E = math.log2(math.e)

UORD = (0, 3, 5, 6, 7, 4, 2, 1)
NSL = 8
DELTA = 2.0
LEADC = 200
LAT_A = 20
LAT_E = 12
LAT_B = 30
AX = 1.5
GA, GB, GO = 3, 2, 2
RES = 44
NBUF = 3
BST = 3
SD0, SDS, SDN, SDJ = 158, 2, 20, 30
QT = 3
RB = 256
PC = 32
P0, PSTEP, PD = 440, 30, 52
NLN, LN0, LNS = 4, 4, 5
LP = 16
PROLOGUE = ('|kva|Z; |b|; kva|wc|K0123; bw|xdn|C0@56 N0123@52 K4567; cx|mq|N4567@52 K89ab; '
            'd|y|C1@56 Kcdef; nmq|zo|M H01 H234567@30 Q0123; y||H89ab@30 Q4567; '
            'zo||L Hcdef@30 Q89ab S01 Qcdef')


def _dot(a, b):
    return jnp.dot(a, b, preferred_element_type=F32)


def _dot_nt(a, b):
    return jax.lax.dot_general(a, b, NT, preferred_element_type=F32)


def _ln(x):
    m = jnp.mean(x, axis=-1, keepdims=True)
    xc = x - m
    v = jnp.mean(xc * xc, axis=-1, keepdims=True)
    return xc * jnp.exp2(jnp.log(v + EPS) * (-0.5 * LOG2E))


def _rows(v, n):
    return jnp.broadcast_to(v[None], (n // 8, 8, v.shape[1])).reshape(n, v.shape[1])


def _gelu(x):
    c0 = math.sqrt(2.0 / math.pi)
    return 0.5 * x * (1.0 + jnp.tanh(c0 * (x + 0.044715 * (x * x * x))))


def _after(x, dep):
    return jnp.where(dep > jnp.inf, dep, x)


def _tie(x, dep):
    xu = pltpu.bitcast(x, U32)
    first = jnp.where(dep > jnp.inf, jnp.uint32(0), xu[:8])
    return pltpu.bitcast(jnp.concatenate([first, xu[8:]], axis=0), BF16)


def _tile(j):
    return slice(j * T, (j + 1) * T)


def _ld(ref, *idx):
    return pltpu.bitcast(ref[idx], BF16)


def _ldb(ref, *idx):
    return pltpu.bitcast(ref.bitcast(U32)[idx], BF16)


def _pk(x):
    return pltpu.bitcast(x, U32)


def _a_ops(a11, a12, a21, a22):
    return [a11 + a22, a21 + a22, a11, a22, a11 + a12, a21 - a11, a12 - a22]


def _b_ops(b11, b12, b21, b22):
    return [b11 + b22, b11, b12 - b22, b21 - b11, b22, b11 + b12, b21 + b22]


def _strassen(prod, col1=None, col2=None):
    m4 = prod(3)
    m2 = prod(1)
    c21 = m2 + m4
    if col1 is not None:
        e11, e21 = col1()
        m4, c21 = m4 + e11, c21 + e21
    m3 = prod(2)
    m5 = prod(4)
    c12 = m3 + m5
    if col2 is not None:
        e12, e22 = col2()
        c12, m3 = c12 + e12, m3 + e22
    m1 = prod(0)
    c11 = prod(6) + (m1 + (m4 - m5))
    c22 = prod(5) + (m1 + (m3 - m2))
    return c11, c12, c21, c22


def _group(rows, cols, pairs):
    xs, ys = dict.fromkeys(x for x, _ in pairs), dict.fromkeys(y for _, y in pairs)
    used = set(xs) | set(ys) | {(x[0], y[1]) for x, y in pairs} | {(y[0], x[1]) for x, y in pairs}
    prods = []
    for n, r in enumerate(rows):
        for i, k in [x for x in xs if x[0] == r]:
            mates = [y for x, y in pairs if x == (i, k)]
            prods.append((((1, i, k),) + tuple((1, i, k2) for _, k2 in mates), ((1, k, 0),),
                          ((1, i, 0), (-1, i, 1))))
            prods.append((((1, i, k),) + tuple((-1, i2, k) for i2, _ in mates), ((1, k, 0), (1, k, 1)),
                          ((1, i, 1),)))
        for i2, k2 in [y for y in ys if y[0] == r]:
            mates = [x for x, y in pairs if y == (i2, k2)]
            prods.append((((1, i2, k2),) + tuple((1, i2, k) for _, k in mates), ((1, k2, 1),),
                          ((1, i2, 1), (-1, i2, 0))))
            prods.append((((1, i2, k2),) + tuple((-1, i, k2) for i, _ in mates), ((1, k2, 0), (1, k2, 1)),
                          ((1, i2, 0),)))
        prods += [(((1, r, k),), ((1, k, h),), ((1, r, h),)) for k in cols if (r, k) not in used for h in (0, 1)]
        for (i, k), (i2, k2) in pairs:
            if r in (i, i2) and i + i2 - r in rows[n + 1:]:
                prods.append((((1, i, k2),), ((1, k2, 0), (-1, k, 0)), ((1, i2, 0), (1, i, 0))))
                prods.append((((1, i2, k), (1, i, k2)), ((1, k, 0), (1, k2, 1)), ((1, i2, 0), (1, i, 1))))
                prods.append((((1, i2, k),), ((1, k, 1), (-1, k2, 1)), ((1, i2, 1), (1, i, 1))))
    return prods


def _all_pairs(xrows, yrows):
    return [((x, a), (y, b)) for a, x in enumerate(xrows) for b, y in enumerate(yrows) if a != b]


_PAIRS65 = [((x[0] + 10, x[1]), (y[0] + 10, y[1])) for x, y in (
    ((0, 1), (1, 0)), ((0, 1), (5, 2)), ((2, 3), (1, 0)), ((2, 3), (3, 1)), ((2, 3), (5, 2)), ((3, 2), (1, 0)),
    ((4, 4), (0, 3)), ((4, 4), (1, 0)), ((4, 4), (3, 1)), ((4, 4), (5, 2)))]
_C_GROUPS = [_group(range(r, r + 8), range(4), _all_pairs(range(r, r + 4), range(r + 4, r + 8))) for r in (0, 8)]
_H_GROUPS = [_group(range(10), range(5), _all_pairs(range(5), range(5, 10))),
             _group(range(10, 16), range(5), _PAIRS65)]
_sum_index = lambda groups: {f: n for n, f in enumerate(
    dict.fromkeys(t[0] for g in groups for t in g if len(t[0]) > 1))}
_C_SUMS, _H_SUMS = _sum_index(_C_GROUPS), _sum_index(_H_GROUPS)


def _form(form, get):
    acc = None
    for sign, i, j in form:
        v = get(i, j)
        acc = v if acc is None else (acc + v if sign > 0 else acc - v)
    return acc


def _gap_items(bufs, gap_scr):
    items = []
    for n, buf in enumerate(bufs):
        acc = []

        def part(r0, buf=buf, acc=acc):
            def fn(dep):
                wu = jnp.concatenate([buf[r:r + 8, :] for r in range(r0, r0 + T, 32)])
                mask = jnp.full((8, T), 0x7FFF0000, U32)
                if dep is not None:
                    mask = jnp.where(dep > jnp.inf, jnp.uint32(0), mask)
                mask = _rows(mask, 32)
                new = [jnp.sum(pltpu.bitcast(v & mask, F32).reshape(4, 8, T), axis=0) for v in (wu << 16, wu)]
                acc[:] = [u + v for u, v in zip(acc, new)] if acc else new
            return fn

        def last(_, n=n, acc=acc):
            bits = []
            for v in acc:
                l1 = jnp.sum(jnp.sum(v, axis=1, keepdims=True), axis=0, keepdims=True)
                bits.append(pltpu.bitcast(jnp.broadcast_to(l1, (8, T)), jnp.int32) >> 8)
            gap_scr[n] = jnp.clip((bits[0] - bits[1] + (1 << 14)) >> 15, -8, 8) << 23

        items += [part(r0) for r0 in range(0, buf.shape[0], T)] + [last]
    return items


class _PairWeights:
    def __init__(self, w_ref, transpose=False, shift=None):
        self.base = {}
        if shift is not None:
            fac = _rows(pltpu.bitcast(0x3F800000 + shift, F32), T)
            self.inv = pltpu.bitcast(0x3F800000 - shift, F32)
        for j in range(w_ref.shape[0] // T):
            wu = w_ref[_tile(j), :]
            if transpose:
                wu = wu.T
            hi = pltpu.bitcast(wu & jnp.uint32(0xFFFF0000), F32)
            self.base[j, 0] = pltpu.bitcast(wu << 16, F32)
            self.base[j, 1] = hi if shift is None else hi * fac
        self.cache = {}

    def __call__(self, form):
        sign = 1
        if form[-1][0] < 0 and form[0][1:] > form[1][1:]:
            sign, form = -1, ((1,) + form[1][1:], (-1,) + form[0][1:])
        if form not in self.cache:
            self.cache[form] = _form(form, lambda k, h: self.base[k, h]).astype(BF16)
        return sign, self.cache[form]


def _run_group(jobs, prods, a_get, w, transposed, finish):
    left = {}
    for _, _, outs in prods:
        for _, i, h in outs:
            left[i, h] = left.get((i, h), 0) + 1
    acc = {}
    for af, bf, outs in prods:
        sign, wt = w(bf)
        m = jobs.mm([wt], [a_get(af)], _dot_nt) if transposed else jobs.mm([a_get(af)], [wt], _dot)
        for s_, i, h in outs:
            if (i, h) not in acc:
                acc[i, h] = (s_ * sign, m)
            else:
                s0, v = acc[i, h]
                acc[i, h] = (s0, v + m if s0 == s_ * sign else v - m) if s0 > 0 or s_ * sign < 0 else (1, m - v)
            left[i, h] -= 1
            if not left[i, h]:
                s0, v = acc.pop((i, h))
                assert s0 > 0
                finish(2 * i + h, v)


class _Jobs:
    def __init__(self, side=()):
        self.res = []
        self.side = list(side)

    def mm(self, lhs, wt, dot):
        acc = None
        for x, w in zip(lhs, wt):
            v = dot(x, w)
            self.res.append(v)
            acc = v if acc is None else v + acc
            rel = 4 * (len(self.res) % 4)
            while self.side and self.side[0][0] <= len(self.res):
                self.side.pop(0)[1](v[8 * rel:8 * rel + 8, :])
                rel = (rel + 2) % 16
        return acc


def _proj_step(h_scr, hs_scr, c_ref, cs_scr, wq_ref, wuk_ref, wuv_ref, q_scr, k_scr, v_scr, scale, shifts, side):
    wk, wvT, wq = [_PairWeights(w, n == 1, shifts[n]) for n, w in enumerate((wuk_ref, wuv_ref, wq_ref))]
    c_get = lambda f: _ldb(cs_scr, _C_SUMS[f]) if len(f) > 1 else c_ref[_tile(f[0][1]), _tile(f[0][2])]
    h_get = lambda f: _ldb(hs_scr, _H_SUMS[f]) if len(f) > 1 else _ldb(h_scr, f[0][1], f[0][2])

    def put(dst, w, mul=None):
        muls = [mul, _rows(w.inv if mul is None else w.inv * mul, T)]

        pend = {}

        def fn(u, v):
            v = (v if muls[u % 2] is None else v * muls[u % 2])
            if dst is v_scr:
                return _v_put(v_scr, pend, u // 2, u % 2, v)
            v = v.astype(BF16)
            dst[u] = v.T if mul is not None and u < QT else v
        return fn

    jobs = _Jobs(side)
    for groups, get, w, transposed, fin in ((_C_GROUPS, c_get, wk, False, put(k_scr, wk)),
                                            (_C_GROUPS, c_get, wvT, True, put(v_scr, wvT)),
                                            (_H_GROUPS, h_get, wq, False, put(q_scr, wq, scale))):
        for prods in groups:
            _run_group(jobs, prods, get, w, transposed, fin)
    assert not jobs.side


def _inner_group(rows, cols, pairs):
    xs, ys = dict.fromkeys(x for x, _ in pairs), dict.fromkeys(y for _, y in pairs)
    used = set(xs) | set(ys) | {(x[0], y[1]) for x, y in pairs} | {(y[0], x[1]) for x, y in pairs}
    prods = []
    for i, j in xs:
        mates = [y for x, y in pairs if x == (i, j)]
        prods.append((((1, i, 0),), ((1, 0, j), (-1, 1, j)), ((1, i, j),) + tuple((1, i2, j) for i2, _ in mates)))
        prods.append((((1, i, 0), (1, i, 1)), ((1, 1, j),), ((1, i, j),) + tuple((-1, i, j2) for _, j2 in mates)))
    for i2, j2 in ys:
        mates = [x for x, y in pairs if y == (i2, j2)]
        prods.append((((1, i2, 0), (1, i2, 1)), ((1, 0, j2),),
                      ((1, i2, j2),) + tuple((-1, i2, j) for _, j in mates)))
        prods.append((((1, i2, 1),), ((1, 0, j2), (-1, 1, j2)),
                      ((-1, i2, j2),) + tuple((-1, i, j2) for i, _ in mates)))
    prods += [(((1, i, h),), ((1, h, j),), ((1, i, j),))
              for i in rows for j in cols if (i, j) not in used for h in (0, 1)]
    for (i, j), (i2, j2) in pairs:
        lo, hi = min(j, j2), max(j, j2)
        prods.append((((1, i2, 0), (-1, i, 0)), ((1, 0, lo), (1, 0, hi)), ((1, i2, j),)))
        prods.append((((1, i, 0), (1, i2, 1)), ((1, 0, j2), (1, 1, j)), ((1, i, j2), (1, i2, j))))
        prods.append((((1, i, 1), (-1, i2, 1)), ((1, 1, lo), (1, 1, hi)), ((1, i, j2),)))
    return prods


def _o_jobs():
    prods = (_inner_group(range(10), range(5), _all_pairs(range(0, 10, 2), range(1, 10, 2)))
             + _inner_group(range(10, 16), range(5), _PAIRS65))
    need = lambda t: max(2 * (i // 2) + h for _, i, h in t[0])
    return [(need(t), t) for t in sorted(prods, key=need)]


_O_JOBS = _o_jobs()


def _job_order(nb):
    size = dict(a=2, b=1, d=2, o=2, e=0)
    qa, qe, qb = [], [], []
    for n in range(nb):
        a = UORD[n // 2]
        qa += [('a', n, (qi, c)) for c in range(2 * a + 2) for qi in range(2) if c <= 2 * a + qi]
        qe += [('e', n, (blk, sl)) for blk in range(a + 1) for sl in range(NSL)]
        qb += [('b', n, (m, blk)) for m in (3, 1, 2, 4, 0, 6, 5) for blk in range(a)]
        qb += [('d', n, j) for j in range(3)]
    qo = [('o', u, j) for j, (u, _) in enumerate(_O_JOBS)]
    qs = dict(a=qa, b=qb, o=qo, e=qe)
    done, order = {}, []
    now, next_e = 0, 0.0
    free = [0] * 4
    pops = []

    def emit(k):
        nonlocal now
        job = qs[k].pop(0)
        if k == 'e':
            _, nj, row = min(pops, key=lambda p: abs(p[0] - (next_e * 16 - LEADC)))
            job = job[:2] + (job[2] + (nj, row),)
        else:
            x = free.index(min(free))
            nj = sum(1 for j in order if j[0] != 'e')
            pops.extend((free[x] + 16 * g, nj, 16 * g) for g in range(4 * size[job[0]]))
            del pops[:-64]
            free[x] += 64 * size[job[0]]
        order.append(job)
        now += size[job[0]]
        if not qs[k] or qs[k][0][1] != job[1]:
            done[k, job[1]] = now

    def ok(k):
        if not qs[k]:
            return False
        n = qs[k][0][1]
        if k == 'a':
            return not qe or n - qe[0][1] < NBUF
        if k == 'e' and qb and n - qb[0][1] >= NBUF:
            return False
        prev, lat = dict(e=('a', LAT_A), b=('e', LAT_E), o=('b', LAT_B))[k]
        return (prev, n) in done and done[prev, n] + lat <= now

    def try_e():
        nonlocal next_e
        if ok('e') and next_e <= now:
            emit('e')
            next_e = max(next_e, now - 1) + DELTA
            return True

    while qa or qe or qb or qo:
        if try_e():
            continue
        cand = [k for k in 'abo' if ok(k)]
        if 'o' in cand and len(qo) <= RES and (qa or 'b' in cand):
            cand.remove('o')
        k = None
        if qe:
            ne = qe[0][1]
            n_e = (UORD[ne // 2] + 1) * NSL
            start = max(done.get(('e', ne - 1), 0), next_e - (n_e - sum(1 for j in qe if j[1] == ne)) * DELTA)
            dur = n_e * DELTA
            fa = 1 - sum(2 for j in qa if j[1] <= ne + 1) / (2 * (4 * UORD[min(ne + 1, nb - 1) // 2] + 3))
            fb = 1 - sum(size[j[0]] for j in qb if j[1] <= ne - 1) / (7 * UORD[max(ne - 1, 0) // 2] + 6)
            due = [((now - start + LAT_A * AX) / dur - fa, 'a'), ((now - start - LAT_E) / max(dur - LAT_E, 1) - fb, 'b')]
            best = max(due, key=lambda x: x[0] if x[1] in cand else -9)
            if best[1] in cand and best[0] > 0:
                k = best[1]
        if k is None:
            k = next((k for k in 'oab' if k in cand), None)
        if k:
            for _ in range(dict(a=GA, b=GB, o=GO)[k]):
                if ok(k):
                    emit(k)
                    try_e()
        else:
            now += 1
    return order


def _attention_step(q_scr, k_scr, v_scr, wo_ref, acc_scr, s_scr, f_scr, zero):
    causal = (jax.lax.broadcasted_iota(jnp.int32, (T, T), 0)
              <= jax.lax.broadcasted_iota(jnp.int32, (T, T), 1))
    mx, mfin, lsum, of, lhs = {}, {}, {}, {}, {}
    macc, dacc, left_b = {}, {}, {}
    res = []
    wo, terms = {}, {}
    left = {}
    for _, t in _O_JOBS:
        for _, i, j in t[2]:
            left[i, j] = left.get((i, j), 0) + 1
    H2 = T // 2

    def job_a(n, j):
        qi, c = j
        r, hd = 2 * UORD[n // 2] + qi, n % 2
        u = 2 * r + hd
        s = (_dot if u < QT else _dot_nt)(_ldb(k_scr, 2 * c + hd), _ldb(q_scr, u))
        res.append(s)
        if c == r:
            s = jnp.where(causal, s, -1e9 * LOG2E)
        s_scr[n % NBUF][zero + 2 * c + qi] = s
        pm = jnp.max(s.reshape(T // 8, 8, T), axis=0)
        mx[n, qi] = pm if (n, qi) not in mx else jnp.maximum(mx[n, qi], pm)

    def row_max(n, qi):
        m = jnp.broadcast_to(jnp.max(mx[n, qi], axis=0, keepdims=True), (8, T))
        if UORD[n // 2] == 0:
            return m
        nt = 2 * UORD[n // 2] + qi + 1
        cs = range(qi % BST, nt, BST)
        es = [jnp.exp2(s_scr[n % NBUF][2 * c + qi, 0:8, :] - m) for c in cs]
        while len(es) > 1:
            es = [es[i] + es[i + 1] if i + 1 < len(es) else es[i] for i in range(0, len(es), 2)]
        est = jnp.maximum(jnp.sum(es[0], axis=0, keepdims=True) * (16.0 * nt / len(cs)), 1.0)
        return m + jnp.log(est) * (0.5 * LOG2E)

    def job_e(n, j):
        blk, sl, nj, r0 = j
        rows = slice(sl * T // NSL, (sl + 1) * T // NSL)
        ms = []
        for qi in range(2):
            if (n, qi) not in mfin:
                mfin[n, qi] = row_max(n, qi)
            ms.append(_after(mfin[n, qi], res[nj][r0:r0 + 8, :]))

        def exps(qi, c):
            p = jnp.exp2(s_scr[n % NBUF][2 * c + qi, rows, :].reshape(-1, 8, T) - ms[qi][None])
            ls = jnp.sum(p, axis=0)
            lsum[n, qi] = ls if (n, qi) not in lsum else lsum[n, qi] + ls
            return p.reshape(-1, T)

        if blk == UORD[n // 2]:
            ops = [exps(qi, 2 * blk + kk) for qi, kk in ((0, 0), (1, 0), (1, 1))]
        else:
            ops = _b_ops(*[exps(qi, 2 * blk + kk) for kk in range(2) for qi in range(2)])
        for i, v in enumerate(ops):
            f_scr[n % NBUF][zero + blk, i, rows, :] = v.astype(BF16)

    def finish(n):
        left_b[n] = left_b.get(n, 7 * UORD[n // 2] + 3) - 1
        if left_b[n]:
            return
        d0, d1 = dacc[n, 0], dacc[n, 1]
        if UORD[n // 2]:
            c11, c12, c21, c22 = _strassen(lambda i: macc[n, i], lambda: (d0[:H2], d0[H2:]),
                                           lambda: (d1[:H2], d1[H2:]))
            d0, d1 = jnp.concatenate([c11, c21], axis=0), jnp.concatenate([c12, c22], axis=0)
        for qi, d in enumerate((d0, d1)):
            of[2 * (2 * (n // 2) + qi) + n % 2] = d * (1.0 / jnp.sum(lsum[n, qi], axis=0, keepdims=True))

    def job_b(n, j):
        m, blk = j
        v = _dot(_ldb(v_scr, n % 2, blk, m), _ldb(f_scr[n % NBUF], blk, m))
        res.append(v)
        macc[n, m] = v if (n, m) not in macc else v + macc[n, m]
        finish(n)

    def job_d(n, j):
        a, vu = UORD[n // 2], v_scr.bitcast(U32)
        i0, i1 = ((2, 7), (2, 7), (8, 3))[j]
        vt = pltpu.bitcast(jnp.concatenate([vu[n % 2, a, i0], vu[n % 2, a, i1]], axis=0), BF16)
        v = _dot(vt, _ldb(f_scr[n % NBUF], a, j))
        res.append(v)
        dacc[n, min(j, 1)] = v if (n, min(j, 1)) not in dacc else v + dacc[n, min(j, 1)]
        finish(n)

    def job_o(_, n):
        af, bf, outs = _O_JOBS[n][1]
        if af not in lhs:
            v = _form(af, lambda i, h: of[2 * i + h])
            lhs[af] = _tie(v.astype(BF16).T, v[0:8, :])
        if bf not in wo:
            wo[bf] = (wo_ref[_tile(bf[0][1]), _tile(bf[0][2])] if len(bf) == 1 else
                      _form(bf, lambda h, j: wo_ref[_tile(h), _tile(j)].astype(F32)).astype(BF16))
        v = _dot(lhs[af], wo[bf])
        res.append(v)
        for sign, i, j in outs:
            terms.setdefault((i, j), []).append((sign, v))
            if len(terms[i, j]) == left[i, j]:
                rows = _tile(2 * UORD[i // 2] + i % 2)
                tot = acc_scr[rows, _tile(j)]
                for sg, m in terms.pop((i, j)):
                    tot = tot + m if sg > 0 else tot - m
                acc_scr[rows, _tile(j)] = tot

    fns = dict(a=job_a, e=job_e, b=job_b, d=job_d, o=job_o)
    for kind, u, j in _job_order(q_scr.shape[0] // 2):
        fns[kind](u, j)


def _v_put(v_scr, pend, i, hd, v):
    pend[i, hd] = v
    if (i ^ 1, hd) in pend:
        lo, hi = pend.pop((i & ~1, hd)), pend.pop((i | 1, hd))
        H2 = T // 2
        a11, a12, a21, a22 = lo[:H2], hi[:H2], lo[H2:], hi[H2:]
        for m, x in enumerate(_a_ops(a11, a12, a21, a22) + [a21, a12]):
            v_scr[hd, i // 2, m] = x.astype(BF16)


def _kernel(x_hbm, c_hbm, wq_hbm, wuk_hbm, wuv_hbm, wo_hbm, w1_hbm, w2_hbm, w3_hbm, w4_hbm,
            cond_hbm, wmod_hbm, out_hbm,
            x_ref, c_ref, cond_ref, wma_ref, wmb_ref, w1_ref, w2_ref, w3_ref, w4_ref,
            wq_buf, wk_buf, wv_buf, wo_buf, out_buf, sem, wsem, osem,
            mod_scr, h_scr, cs_scr, hs_scr, w_scr, q_scr, k_scr, v_scr, acc_scr, xn_scr, xh_scr, a1_scr, t_scr,
            ws12, ws3, ws4, pq_buf, pk_buf, pv_buf, gap_scr, st_in, *rest):
    f_scr, s_scr = rest[:NBUF], rest[NBUF:]
    S, M = x_hbm.shape
    D = wq_hbm.shape[2]
    nattn = wo_hbm.shape[0]
    Fd = w4_hbm.shape[0]
    scale = float(D) ** -0.5 * LOG2E
    nb, nrb = S // T, S // RB
    km, kc = M // T, c_hbm.shape[1] // T
    NX = 4
    XR = S // NX
    CB = XR // T

    work, probe = (wk_buf, wv_buf, wq_buf), (pk_buf, pv_buf, pq_buf)

    def pcopies(g, bufs=work, s0=0):
        return [pltpu.make_async_copy(src.bitcast(U32).at[:, g, :], dst, wsem.at[s0 + j])
                for j, (src, dst) in enumerate(zip((wuk_hbm, wuv_hbm, wq_hbm), bufs))]

    def ocopy(g):
        return pltpu.make_async_copy(wo_hbm.at[g], wo_buf, wsem.at[3])

    def chunk_copy(src, dst, i, s0):
        rows = slice(i * XR, (i + 1) * XR)
        return pltpu.make_async_copy(src.at[rows, :], dst.at[rows, :], sem.at[s0 + i])

    cp_cond = pltpu.make_async_copy(cond_hbm, cond_ref, sem.at[0])
    cp_wma = pltpu.make_async_copy(wmod_hbm.at[:, 0:2 * M], wma_ref, sem.at[1])
    cp_late = [pltpu.make_async_copy(src, dst, sem.at[2 + j]) for j, (src, dst) in enumerate((
        (wmod_hbm.at[:, 2 * M:6 * M], wmb_ref), (w1_hbm, w1_ref), (w2_hbm, w2_ref),
        (w3_hbm, w3_ref), (w4_hbm, w4_ref)))]
    cp_x = [chunk_copy(x_hbm, x_ref, i, 7) for i in range(NX)]
    cp_c = [chunk_copy(c_hbm, c_ref, i, 7 + NX) for i in range(NX)]

    def silu_cond():
        cf = cond_ref[...].astype(F32)
        return jnp.broadcast_to((cf * jax.nn.sigmoid(cf)).astype(BF16), (8, M))

    cp_wk, cp_wv, cp_wq = pcopies(0)
    named = dict(k=cp_wk, v=cp_wv, q=cp_wq, o=ocopy(0), n=cp_cond, m=cp_wma)
    named.update(zip('abcd', cp_c))
    named.update(zip('wxyz', cp_x))
    started, arrived, did = set(), set(), set()
    vpend = {}

    def zero(r, carry):
        acc_scr[pl.ds(pl.multiple_of(r * T, T), T), :] = jnp.zeros((T, M), F32)
        return carry

    def x_rows(rows, dep):
        xf = x_ref[rows, :].astype(F32)
        if dep is None:
            return xf
        return jnp.concatenate([_after(xf[:, :T], _rows(dep, xf.shape[0])), xf[:, T:]], axis=1)

    def n_item(r, i):
        def fn(dep):
            rows = slice(r * T + i * LP, r * T + (i + 1) * LP)
            xn_scr[rows, :] = _ln(x_rows(rows, dep))
        return fn

    def h_item(r, i, normed):
        def fn(dep):
            rows = slice(i * LP, (i + 1) * LP)
            grows = slice(r * T + i * LP, r * T + (i + 1) * LP)
            sa = mod_scr[:, 0:M]
            if normed and dep is not None:
                sa = jnp.concatenate([_after(sa[:, _tile(j)], dep) for j in range(km)], axis=1)
            hf = ((xn_scr[grows, :] if normed else _ln(x_rows(grows, dep))) * _rows(mod_scr[:, M:2 * M], LP)
                  + _rows(sa, LP))
            for j in range(km):
                h_scr[r, j, rows, :] = hf[:, _tile(j)].astype(BF16)
            for f, n in _H_SUMS.items():
                if all(t[1] == r for t in f):
                    hs_scr[n, rows, :] = _form(f, lambda _, k: hf[:, _tile(k)]).astype(BF16)
            did.add(('h', r, i))
        return fn

    def release(jobs, span, items):
        if span and items:
            jobs.side += [(len(jobs.res) + 1 + i * span // len(items), fn) for i, fn in enumerate(items)]
            jobs.side.sort(key=lambda e: e[0])
        else:
            for fn in items:
                fn(None)

    def sum_items(n, group, index, dst, get, skip_rows):
        forms = [f for f in dict.fromkeys(t[0] for t in group)
                 if len(f) > 1 and not (skip_rows and len({t[1] for t in f}) == 1)]

        def item(f, rows):
            def fn(dep):
                def term(r, k):
                    v = get(r, k, rows).astype(F32)
                    return v if dep is None or (r, k) != f[0][1:] else _after(v, _rows(dep, v.shape[0]))
                dst[index[f], rows, :] = _form(f, term).astype(BF16)
            return fn

        return [item(f, slice(i, i + n)) for i in range(0, T, n) for f in forms]

    h_sums = lambda n, gi: sum_items(n, _H_GROUPS[gi], _H_SUMS, hs_scr,
                                     lambda r_, k, rows: h_scr[r_, k, rows, :], True)

    def stash(key, buf, j0, transpose=False):
        n = buf.shape[0] // T
        if key not in did:
            assert key in arrived
            did.add(key)
            w = _PairWeights(buf, transpose)
            for j in range(n):
                for hd in range(2):
                    w_scr[hd, j0 + j] = w(((1, j, hd),))[1]
        return lambda hd: [_ldb(w_scr, hd, j0 + j) for j in range(n)]

    def kv_tile(jobs, r):
        wk, wvT = stash('k', wk_buf, 0), stash('v', wv_buf, kc, True)
        ct = [c_ref[_tile(r), _tile(j)] for j in range(kc)]
        for hd in range(2):
            k_scr[2 * r + hd] = jobs.mm(ct, wk(hd), _dot).astype(BF16)
        for hd in range(2):
            _v_put(v_scr, vpend, r, hd, jobs.mm(wvT(hd), ct, _dot_nt))

    def q_tile(jobs, r):
        wq = stash('q', wq_buf, 2 * kc)
        ht = [_ldb(h_scr, r, j) for j in range(km)]
        for hd in range(2):
            v = (jobs.mm(ht, wq(hd), _dot) * scale).astype(BF16)
            q_scr[2 * r + hd] = v.T if 2 * r + hd < QT else v

    for blk in PROLOGUE.split(';'):
        waits, starts, acts = blk.split('|')
        for ch in waits.strip():
            assert ch in started and ch not in arrived
            arrived.add(ch)
            named[ch].wait()
        for ch in starts.strip():
            assert ch not in started
            started.add(ch)
            named[ch].start()
        jobs = _Jobs()
        for act in acts.split():
            if act == 'Z':
                jax.lax.fori_loop(0, nb, zero, 0)
                acc_scr[S:, :] = jnp.zeros((acc_scr.shape[0] - S, M), F32)
                x_ref[S:, :] = jnp.zeros((x_ref.shape[0] - S, M), BF16)
            elif act == 'L':
                did.add('L')
                for cp in cp_late:
                    cp.start()
            elif act == 'M':
                assert arrived >= set('nm')
                mod = _dot(silu_cond(), wma_ref[...])
                mod_scr[:, 0:M] = mod[:, 0:M]
                mod_scr[:, M:2 * M] = 1.0 + mod[:, M:2 * M]
                did.add('M')
            else:
                act, _, span = act.partition('@')
                span = int(span or 0)
                items = []
                for r in [int(ch, 16) for ch in act[1:]]:
                    did.add((act[0], r))
                    if act[0] == 'K':
                        assert 'abcd'[r // CB] in arrived
                        kv_tile(jobs, r)
                    elif act[0] == 'H':
                        assert 'wxyz'[r // CB] in arrived and 'M' in did
                        items += [h_item(r, i, ('N', r) in did) for i in range(T // LP)]
                    elif act[0] == 'N':
                        assert 'wxyz'[r // CB] in arrived
                        items += [n_item(r, i) for i in range(T // LP)]
                    elif act[0] == 'Q':
                        assert all(('h', r, i) in did for i in range(T // LP))
                        q_tile(jobs, r)
                    elif act[0] == 'C':
                        assert all('abcd'[t[1] // CB] in arrived for p_ in _C_GROUPS[r] for t in p_[0])
                        items += sum_items(
                            32, _C_GROUPS[r], _C_SUMS, cs_scr,
                            lambda r_, k, rows: c_ref[r_ * T + rows.start:r_ * T + rows.stop, _tile(k)], False)
                    else:
                        assert act[0] == 'S' and all(('h', t[1], T // LP - 1) in did for p_ in _H_GROUPS[r] for t in p_[0])
                        items += h_sums(32 if span else 16, r)
                release(jobs, span, items)
        assert not jobs.side
    assert arrived == set(named) and all((k_, r) in did for k_ in 'KHQ' for r in range(nb))
    assert all((k_, r) in did for k_ in 'CS' for r in range(2)) and 'L' in did

    FH = ws3.shape[0] * T
    assert nattn - 1 >= FH // 64

    slices = ((w1_hbm, 32, 2 * T, 0), (w2_hbm, 32, 2 * T, 64), (w4_hbm, 64, FH, 128), (w3_hbm, T, FH, 256))
    slice_of = lambda g, n, half: jnp.minimum(g, half // n - 1)

    def prep_in(g):
        return [pltpu.make_async_copy(
            w.at[pl.ds(pl.multiple_of(slice_of(g, n, half) * n + x * half, n), n), 0:4 * T],
            st_in.at[r0 + x * n:r0 + (x + 1) * n, :], wsem.at[7]) for w, n, half, r0 in slices for x in range(2)]

    def mixer_prep(g):
        def blocks(r0, n, half, c0, c1, dep):
            get = lambda x, c: st_in[r0 + x * half:r0 + x * half + n, _tile(c)].astype(F32)
            return [_after(get(0, c0), _rows(dep, n)), get(0, c1), get(1, c0), _after(get(1, c1), _rows(dep, n))]

        def rows_item(dst, per, half, r0, c, o, n=16):
            def fn(dep):
                rows = pl.ds(pl.multiple_of(slice_of(g, per, half) * (per // 2), per // 2) + o // 2, n // 2)
                for i, v in enumerate(_b_ops(*blocks(r0 + o, n, per, c, c + 2, dep))):
                    dst[i, c, rows, :] = _pk(v.astype(BF16))
            return fn

        def w3_item(k, i):
            def fn(dep):
                b11, b21, b12, b22 = blocks(slices[3][3], T, T, k, k + 2, dep)
                ws3[slice_of(g, T, FH), i, k] = _pk(_b_ops(b11, b12, b21, b22)[i].astype(BF16).T)
            return fn

        return ([rows_item(dst, *sl[1:], c, o) for dst, sl in zip((ws12.at[0], ws12.at[1], ws4), slices)
                 for c in range(2) for o in range(0, sl[1], 16)]
                + [w3_item(k, i) for k in range(2) for i in range(7)])

    def next_copies(g):
        return pcopies(jnp.minimum(g + 1, nattn - 1)) + pcopies(jnp.minimum(g + 2, nattn - 1), probe, 4)

    for cp in next_copies(0) + prep_in(0):
        cp.start()

    def attn_body(g, carry):
        copies = next_copies(g)

        _attention_step(q_scr, k_scr, v_scr, wo_buf, acc_scr, s_scr, f_scr, jnp.minimum(g, 0))
        for cp in copies:
            cp.wait()
        pltpu.make_async_copy(st_in, st_in, wsem.at[7]).wait()

        @pl.when(g == 0)
        def _():
            for fn in _gap_items(work, gap_scr):
                fn(None)

        @pl.when(g + 1 < nattn)
        def _():
            ocopy(g + 1).start()
            side = mixer_prep(g) + _gap_items(probe, gap_scr)
            side = [(SD0 + i * SDS + (SDJ if i >= SDN else 0), fn) for i, fn in enumerate(side)]
            _proj_step(h_scr, hs_scr, c_ref, cs_scr, wq_buf, wk_buf, wv_buf, q_scr, k_scr, v_scr, scale,
                       gap_scr, side)
            for cp in next_copies(g + 1) + prep_in(g + 1):
                cp.start()
            ocopy(g + 1).wait()

        return carry

    jax.lax.fori_loop(0, nattn, attn_body, 0)

    for cp in cp_late:
        cp.wait()
    mod = _dot(silu_cond(), wmb_ref[...])
    mod_scr[:, 2 * M:4 * M] = mod[:, 0:2 * M]
    mod_scr[:, 4 * M:5 * M] = 1.0 + mod[:, 2 * M:3 * M]
    mod_scr[:, 5 * M:6 * M] = mod[:, 3 * M:4 * M]
    ftiles = [(f, min(f + T, Fd)) for f in range(0, Fd, T)]
    OFF = x_ref.shape[0] - S
    CAR = t_scr.shape[0] - RB

    def p1(r0, l0, n, dep=None):
        ga = mod_scr[:, 2 * M:3 * M]
        if dep is not None:
            ga = jnp.concatenate([_after(ga[:, 0:T], dep), ga[:, T:]], axis=1)
        rows = pl.ds(r0, n)
        x1 = x_ref[rows, :].astype(F32) + _rows(ga, n) * acc_scr[rows, :]
        xh_scr[0, l0:l0 + n, :] = x1
        hb = _ln(x1) * _rows(mod_scr[:, 4 * M:5 * M], n) + _rows(mod_scr[:, 3 * M:4 * M], n)
        xh_scr[1, l0:l0 + n, :] = hb
        return _ln(hb)

    HT = T // 2

    def p1_store(r0, c, dep=None):
        v = p1(r0 + c * PC, OFF + c * PC, PC, dep)
        a1_scr[c * PC:(c + 1) * PC, :] = v
        return jnp.max(v[:, M - T:].reshape(PC // 8, 8, T), axis=0)

    t_scr[RB:RB + CAR - OFF, :] = jnp.zeros((CAR - OFF, M), F32)
    t_scr[RB + CAR - OFF:RB + CAR, :] = _gelu(_dot(p1(0, 0, OFF).astype(BF16), w1_ref[...]))
    for c in range(RB // PC):
        p1_store(OFF, c)

    def out_copy(i):
        rows = pl.ds(i * T if isinstance(i, int) else pl.multiple_of(i * T, T), T)
        return pltpu.make_async_copy(out_buf.at[rows, :], out_hbm.at[rows, :], osem.at[i])

    def b_body(r, carry):
        gb = _rows(mod_scr[:, 5 * M:6 * M], T)
        r0 = pl.multiple_of(r * RB, RB)
        n0 = pl.multiple_of(jnp.minimum(r0 + RB, S - RB) + OFF, OFF)
        nh = RB // T
        now = [0]
        due = []
        pace = []

        def p1_item(c):
            return lambda dep: due.append((now[0] + PD, p1_store(n0, c, dep)))

        pace += [(P0 + i * PSTEP, p1_item(i)) for i in range(RB // PC)]
        wt = lambda ref, f0, f1, n: ref[f0:f1, _tile(n)]

        def mm(lhs, wts, dot=_dot):
            acc = None
            for x, w in zip(lhs, wts):
                if due and due[0][0] <= now[0]:
                    w = _tie(w, due.pop(0)[1])
                v = dot(x, w)
                now[0] += x.shape[0] // HT
                acc = v if acc is None else v + acc
                if pace and pace[0][0] <= now[0]:
                    pace.pop(0)[1](v[0:8, :])
            return acc

        def split_ops(lo, hi):
            return [v.astype(BF16) for v in _a_ops(lo[:HT], hi[:HT], lo[HT:], hi[HT:])]

        def two_tiles(aops, wsel, rest):
            def col(w):
                v = mm(rest[0], w, rest[3])
                return v[:HT], v[HT:]

            c11, c12, c21, c22 = _strassen(
                lambda i: mm([a[i] for a in aops], [wsel(i, k) for k in range(len(aops))]),
                lambda: col(rest[1]), lambda: col(rest[2]))
            return jnp.concatenate([c11, c21], axis=0), jnp.concatenate([c12, c22], axis=0)

        def square(full, aops, w_ref, ws_ref):
            out = {}
            for n in range(2):
                out[n], out[n + 2] = two_tiles(
                    aops, lambda i, k: _ld(ws_ref, i, n, slice(k * HT, (k + 1) * HT)),
                    (full[4:], [wt(w_ref, 4 * T, M, n)], [wt(w_ref, 4 * T, M, n + 2)], _dot))
            out[4] = mm(full, [wt(w_ref, j * T, (j + 1) * T, 4) for j in range(km)])
            return out

        t_scr[0:CAR, :] = t_scr[RB:RB + CAR, :]
        for hf in range(nh):
            a1 = [a1_scr[_tile(hf), _tile(j)] for j in range(km)]
            full = [v.astype(BF16) for v in a1]
            aops = [split_ops(a1[k], a1[2 + k]) for k in range(2)]
            for n, v in square(full, aops, w1_ref, ws12.at[0]).items():
                t = _gelu(v)
                if hf == nh - 1:
                    t = jnp.concatenate([t[:T - OFF], jnp.where(r < nrb - 1, t[T - OFF:], 0.0)], axis=0)
                t_scr[CAR + hf * T:CAR + (hf + 1) * T, _tile(n)] = t
        cq = M // 4
        shifts = (-1, 1, -2, 2)
        lane = jax.lax.broadcasted_iota(jnp.int32, (T, T), 1)
        y1, z, a3 = [], [], []
        for hf in range(nh):
            base = CAR - OFF + hf * T
            sh = []
            for j in range(km):
                g_lo, g_hi = (j * T) // cq, ((j + 1) * T - 1) // cq
                assert g_hi - g_lo <= 1
                v = t_scr[base + shifts[g_lo]:base + shifts[g_lo] + T, _tile(j)]
                if g_hi != g_lo:
                    v2 = t_scr[base + shifts[g_hi]:base + shifts[g_hi] + T, _tile(j)]
                    v = jnp.where(lane < g_hi * cq - j * T, v, v2)
                sh.append(v)
            hs = square([v.astype(BF16) for v in sh], [split_ops(sh[k], sh[2 + k]) for k in range(2)],
                        w2_ref, ws12.at[1])
            hs = jnp.concatenate([hs[n] for n in range(km)], axis=1)
            y1.append(hs + xh_scr[1, _tile(hf), :])
            z.append(xh_scr[0, _tile(hf), :] + gb * y1[hf])
            a3.append({})

            def ln_item(hf, c):
                def item(dep):
                    n = HT // NLN
                    for d in (0, HT):
                        v = y1[hf][d + c * n:d + (c + 1) * n]
                        if dep is not None:
                            v = jnp.concatenate([_after(v[:, :T], _rows(dep, n)), v[:, T:]], axis=1)
                        a3[hf][d + c * n] = _ln(v)
                return item

            ln_item(hf, 0)(None)
            pace += [(now[0] + LN0 + (c - 1) * LNS * (1 + hf), ln_item(hf, c)) for c in range(1, NLN)]
            pace.sort(key=lambda e: e[0])
        xh_scr[:, 0:OFF, :] = xh_scr[:, RB:RB + OFF, :]
        nf = FH // T
        h3, h3ops = [], []
        for hf in range(nh):
            assert len(a3[hf]) == 2 * NLN
            af = jnp.concatenate([a3[hf][key] for key in sorted(a3[hf])], axis=0)
            full = [af[:, _tile(j)].astype(BF16) for j in range(km)]
            aops = [split_ops(af[:, _tile(k)], af[:, _tile(2 + k)]) for k in range(2)]
            row, ops = {}, []
            narrow = None
            for n in range(nf):
                lo, hi = two_tiles(aops, lambda i, k: _ld(ws3, n, i, k),
                                   (full[4:], [wt(w3_ref, *ftiles[n], 4)],
                                    [wt(w3_ref, *ftiles[nf + n], 4)], _dot_nt))
                lo, hi = _gelu(lo), _gelu(hi)
                row[n], row[nf + n] = lo.astype(BF16), hi.astype(BF16)
                ops.append(split_ops(lo, hi))
                if n < km:
                    v = mm([wt(w3_ref, *ftiles[-1], n)], [full[n]], _dot_nt)
                    narrow = v if narrow is None else v + narrow
            row[2 * nf] = _gelu(mm(full, [wt(w3_ref, *ftiles[2 * nf], j) for j in range(km)],
                                   _dot_nt)).astype(BF16)
            fw = Fd - ftiles[-1][0]
            gT = jnp.concatenate([_gelu(narrow), jnp.zeros((T - fw, T), F32)], axis=0)
            row[2 * nf + 1] = _tie(gT.astype(BF16).T, gT[0:8, :])[:, :fw]
            h3.append([row[i] for i in range(len(ftiles))])
            h3ops.append(ops)
        for hf in range(nh):
            rows = pl.ds(pl.multiple_of(r0 + hf * T, T), T)

            def finish(n, v):
                out_buf[rows, _tile(n)] = (z[hf][:, _tile(n)] + gb[:, _tile(n)] * v).astype(out_buf.dtype)

            w4t = lambda n, f_: [wt(w4_ref, f0, f1, n) for f0, f1 in f_]
            finish(4, mm(h3[hf], w4t(4, ftiles)))
            for n in range(2):
                lo, hi = two_tiles(h3ops[hf], lambda i, k: _ld(ws4, i, n, slice(k * HT, (k + 1) * HT)),
                                   (h3[hf][2 * nf:], w4t(n, ftiles[2 * nf:]), w4t(n + 2, ftiles[2 * nf:]), _dot))
                finish(n, lo)
                finish(n + 2, hi)
            out_copy(r * nh + hf).start()
        assert not pace
        return carry

    jax.lax.fori_loop(0, nrb, b_body, 0)
    for i in range(nb):
        out_copy(i).wait()


@jax.jit
def pallas_adaLN_cond__compressed_kv_cla__mixer_s_mlp__prompt_kernel(
    A_x: jax.Array,
    A_c_kv: jax.Array,
    A_w_q: jax.Array,
    A_w_uk: jax.Array,
    A_w_uv: jax.Array,
    A_w_o: jax.Array,
    B_x: jax.Array,
    B_w1: jax.Array,
    B_w2: jax.Array,
    B_w3: jax.Array,
    B_w4: jax.Array,
    c: jax.Array,
    w_mod: jax.Array,
):
    _, S, M = A_x.shape
    Dc = A_c_kv.shape[2]
    H, D = A_w_q.shape[1], A_w_q.shape[2]
    Fd = B_w3.shape[1]
    assert D == T and A_c_kv.shape[1] == S and Dc == 4 * T and M == 5 * T and 13 * T < Fd < 14 * T and S == 16 * T
    vmem = pltpu.VMEM
    packed = lambda *lead: vmem(lead + (T // 2, T), U32)
    out = pl.pallas_call(
        _kernel,
        in_specs=[pl.BlockSpec(memory_space=pltpu.HBM)] * 12,
        out_specs=pl.BlockSpec(memory_space=pltpu.HBM),
        out_shape=jax.ShapeDtypeStruct((S, M), A_x.dtype),
        scratch_shapes=[
            vmem((S + 16, M), BF16),
            vmem((S, Dc), BF16),
            vmem((1, M), BF16),
            vmem((M, 2 * M), BF16),
            vmem((M, 4 * M), BF16),
            vmem((M, M), BF16),
            vmem((M, M), BF16),
            vmem((Fd, M), BF16),
            vmem((Fd, M), BF16),
            vmem((M, D), U32),
            vmem((Dc, D), U32),
            vmem((Dc, D), U32),
            vmem((2 * D, M), BF16),
            vmem((S, M), A_x.dtype),
            pltpu.SemaphoreType.DMA((15,)),
            pltpu.SemaphoreType.DMA((8,)),
            pltpu.SemaphoreType.DMA((S // T,)),
            vmem((8, 6 * M), F32),
            vmem((S // T, M // T, T, T), BF16),
            vmem((len(_C_SUMS), T, T), BF16),
            vmem((len(_H_SUMS), T, T), BF16),
            vmem((2, M // T + 2 * (Dc // T), T, T), BF16),
            vmem((2 * S // T, T, T), BF16),
            vmem((2 * S // T, T, T), BF16),
            vmem((2, S // T // 2, 9, T // 2, T), BF16),
            vmem((S + 16, M), F32),
            vmem((S, M), F32),
            vmem((2, RB + 16, M), F32),
            vmem((RB, M), F32),
            vmem((RB + 32, M), F32),
            vmem((2, 7, 2, T, T), U32),
            packed(6, 7, 2),
            vmem((7, 2, 3 * T, T), U32),
            vmem((M, D), U32),
            vmem((Dc, D), U32),
            vmem((Dc, D), U32),
            vmem((3, 8, T), jnp.int32),
            vmem((4 * T, 4 * T), BF16),
        ] + [vmem((8, 7, T, T), BF16)] * NBUF + [vmem((32, T, T), F32)] * NBUF,
        compiler_params=pltpu.CompilerParams(
            vmem_limit_bytes=100 * 1024 * 1024,
            disable_bounds_checks=True,
        ),
    )(
        A_x.reshape(S, M), A_c_kv.reshape(S, Dc),
        A_w_q, A_w_uk, A_w_uv,
        A_w_o.reshape(H // 2, 2 * D, M),
        B_w1, B_w2, B_w3.T, B_w4, c, w_mod,
    )
    return out.reshape(1, S, M)
```

```python
import math

import jax
import jax.numpy as jnp
import jax.experimental.pallas as pl
import jax.experimental.pallas.tpu as pltpu

F32 = jnp.float32
BF16 = jnp.bfloat16
U32 = jnp.uint32
NT = (((1,), (1,)), ((), ()))
T = 128
EPS = 1e-5
LOG2E = math.log2(math.e)

UORD = (0, 3, 5, 6, 7, 4, 2, 1)
NSL = 8
DELTA = 2.0
LEADC = 200
LAT_A = 20
LAT_E = 12
LAT_B = 30
AX = 1.5
GA, GB, GO = 3, 2, 2
RES = 44
NBUF = 3
BST = 3
PORD = 'k1k0q0q1v1v0'
SD0, SDS, SDN, SDJ = 158, 1, 20, 30
QT = 3
RB = 256
PC = 32
P0, PSTEP, PD = 440, 30, 52
NLN, LN0, LNS = 4, 4, 5
LP = 16
PROLOGUE = ('|kva|Z; |b|; kva|wc|K0123; bw|xdn|C0@56 N0123@52 K4567; cx|mq|N4567@52 K89ab; '
            'd|y|C1@56 Kcdef; nmq|zo|M H012 H34567@30 Q0123; y||H89ab@34 Q4567; '
            'zo||L Hcdef@30 S0@80 Q89ab S1 Qcdef')


def _dot(a, b):
    return jnp.dot(a, b, preferred_element_type=F32)


def _dot_nt(a, b):
    return jax.lax.dot_general(a, b, NT, preferred_element_type=F32)


def _ln(x):
    m = jnp.mean(x, axis=-1, keepdims=True)
    xc = x - m
    v = jnp.mean(xc * xc, axis=-1, keepdims=True)
    return xc * jnp.exp2(jnp.log(v + EPS) * (-0.5 * LOG2E))


def _rows(v, n):
    return jnp.broadcast_to(v[None], (n // 8, 8, v.shape[1])).reshape(n, v.shape[1])


def _gelu(x):
    c0 = math.sqrt(2.0 / math.pi)
    return 0.5 * x * (1.0 + jnp.tanh(c0 * (x + 0.044715 * (x * x * x))))


def _after(x, dep):
    return jnp.where(dep > jnp.inf, dep, x)


def _tie(x, dep):
    xu = pltpu.bitcast(x, U32)
    first = jnp.where(dep > jnp.inf, jnp.uint32(0), xu[:8])
    return pltpu.bitcast(jnp.concatenate([first, xu[8:]], axis=0), BF16)


def _tile(j):
    return slice(j * T, (j + 1) * T)


def _ld(ref, *idx):
    return pltpu.bitcast(ref[idx], BF16)


def _ldb(ref, *idx):
    return pltpu.bitcast(ref.bitcast(U32)[idx], BF16)


def _pk(x):
    return pltpu.bitcast(x, U32)


def _a_ops(a11, a12, a21, a22):
    return [a11 + a22, a21 + a22, a11, a22, a11 + a12, a21 - a11, a12 - a22]


def _b_ops(b11, b12, b21, b22):
    return [b11 + b22, b11, b12 - b22, b21 - b11, b22, b11 + b12, b21 + b22]


def _strassen(prod, col1=None, col2=None):
    m4 = prod(3)
    m2 = prod(1)
    c21 = m2 + m4
    if col1 is not None:
        e11, e21 = col1()
        m4, c21 = m4 + e11, c21 + e21
    m3 = prod(2)
    m5 = prod(4)
    c12 = m3 + m5
    if col2 is not None:
        e12, e22 = col2()
        c12, m3 = c12 + e12, m3 + e22
    m1 = prod(0)
    c11 = prod(6) + (m1 + (m4 - m5))
    c22 = prod(5) + (m1 + (m3 - m2))
    return c11, c12, c21, c22


def _group(rows, cols, pairs):
    xs, ys = dict.fromkeys(x for x, _ in pairs), dict.fromkeys(y for _, y in pairs)
    used = set(xs) | set(ys) | {(x[0], y[1]) for x, y in pairs} | {(y[0], x[1]) for x, y in pairs}
    prods = []
    for n, r in enumerate(rows):
        for i, k in [x for x in xs if x[0] == r]:
            mates = [y for x, y in pairs if x == (i, k)]
            prods.append((((1, i, k),) + tuple((1, i, k2) for _, k2 in mates), ((1, k, 0),),
                          ((1, i, 0), (-1, i, 1))))
            prods.append((((1, i, k),) + tuple((-1, i2, k) for i2, _ in mates), ((1, k, 0), (1, k, 1)),
                          ((1, i, 1),)))
        for i2, k2 in [y for y in ys if y[0] == r]:
            mates = [x for x, y in pairs if y == (i2, k2)]
            prods.append((((1, i2, k2),) + tuple((1, i2, k) for _, k in mates), ((1, k2, 1),),
                          ((1, i2, 1), (-1, i2, 0))))
            prods.append((((1, i2, k2),) + tuple((-1, i, k2) for i, _ in mates), ((1, k2, 0), (1, k2, 1)),
                          ((1, i2, 0),)))
        prods += [(((1, r, k),), ((1, k, h),), ((1, r, h),)) for k in cols if (r, k) not in used for h in (0, 1)]
        for (i, k), (i2, k2) in pairs:
            if r in (i, i2) and i + i2 - r in rows[n + 1:]:
                prods.append((((1, i, k2),), ((1, k2, 0), (-1, k, 0)), ((1, i2, 0), (1, i, 0))))
                prods.append((((1, i2, k), (1, i, k2)), ((1, k, 0), (1, k2, 1)), ((1, i2, 0), (1, i, 1))))
                prods.append((((1, i2, k),), ((1, k, 1), (-1, k2, 1)), ((1, i2, 1), (1, i, 1))))
    return prods


def _all_pairs(xrows, yrows):
    return [((x, a), (y, b)) for a, x in enumerate(xrows) for b, y in enumerate(yrows) if a != b]


_PAIRS65 = [((x[0] + 10, x[1]), (y[0] + 10, y[1])) for x, y in (
    ((0, 1), (1, 0)), ((0, 1), (5, 2)), ((2, 3), (1, 0)), ((2, 3), (3, 1)), ((2, 3), (5, 2)), ((3, 2), (1, 0)),
    ((4, 4), (0, 3)), ((4, 4), (1, 0)), ((4, 4), (3, 1)), ((4, 4), (5, 2)))]
_C_GROUPS = [_group(range(r, r + 8), range(4), _all_pairs(range(r, r + 4), range(r + 4, r + 8))) for r in (0, 8)]
_H_GROUPS = [_group(range(10), range(5), _all_pairs(range(5), range(5, 10))),
             _group(range(10, 16), range(5), _PAIRS65)]
_sum_index = lambda groups: {f: n for n, f in enumerate(
    dict.fromkeys(t[0] for g in groups for t in g if len(t[0]) > 1))}
_C_SUMS, _H_SUMS = _sum_index(_C_GROUPS), _sum_index(_H_GROUPS)


def _form(form, get):
    acc = None
    for sign, i, j in form:
        v = get(i, j)
        acc = v if acc is None else (acc + v if sign > 0 else acc - v)
    return acc


def _gap_items(bufs, gap_scr):
    items = []
    for n, buf in enumerate(bufs):
        acc = []

        def part(r0, buf=buf, acc=acc):
            def fn(dep):
                wu = jnp.concatenate([buf[r:r + 8, :] for r in range(r0, r0 + T, 32)])
                mask = jnp.full((8, T), 0x7FFF0000, U32)
                if dep is not None:
                    mask = jnp.where(dep > jnp.inf, jnp.uint32(0), mask)
                mask = _rows(mask, 32)
                new = [jnp.sum(pltpu.bitcast(v & mask, F32).reshape(4, 8, T), axis=0) for v in (wu << 16, wu)]
                acc[:] = [u + v for u, v in zip(acc, new)] if acc else new
            return fn

        def last(_, n=n, acc=acc):
            bits = []
            for v in acc:
                l1 = jnp.sum(jnp.sum(v, axis=1, keepdims=True), axis=0, keepdims=True)
                bits.append(pltpu.bitcast(jnp.broadcast_to(l1, (8, T)), jnp.int32) >> 8)
            gap_scr[n] = jnp.clip((bits[0] - bits[1] + (1 << 14)) >> 15, -8, 8) << 23

        items += [part(r0) for r0 in range(0, buf.shape[0], T)] + [last]
    return items


class _PairWeights:
    def __init__(self, w_ref, transpose=False, shift=None):
        self.base = {}
        if shift is not None:
            fac = _rows(pltpu.bitcast(0x3F800000 + shift, F32), T)
            self.inv = pltpu.bitcast(0x3F800000 - shift, F32)
        for j in range(w_ref.shape[0] // T):
            wu = w_ref[_tile(j), :]
            if transpose:
                wu = wu.T
            hi = pltpu.bitcast(wu & jnp.uint32(0xFFFF0000), F32)
            self.base[j, 0] = pltpu.bitcast(wu << 16, F32)
            self.base[j, 1] = hi if shift is None else hi * fac
        self.cache = {}

    def __call__(self, form):
        sign = 1
        if form[-1][0] < 0 and form[0][1:] > form[1][1:]:
            sign, form = -1, ((1,) + form[1][1:], (-1,) + form[0][1:])
        if form not in self.cache:
            self.cache[form] = _form(form, lambda k, h: self.base[k, h]).astype(BF16)
        return sign, self.cache[form]


def _run_group(jobs, prods, a_get, w, transposed, finish):
    left = {}
    for _, _, outs in prods:
        for _, i, h in outs:
            left[i, h] = left.get((i, h), 0) + 1
    acc = {}
    for af, bf, outs in prods:
        sign, wt = w(bf)
        m = jobs.mm([wt], [a_get(af)], _dot_nt) if transposed else jobs.mm([a_get(af)], [wt], _dot)
        for s_, i, h in outs:
            if (i, h) not in acc:
                acc[i, h] = (s_ * sign, m)
            else:
                s0, v = acc[i, h]
                acc[i, h] = (s0, v + m if s0 == s_ * sign else v - m) if s0 > 0 or s_ * sign < 0 else (1, m - v)
            left[i, h] -= 1
            if not left[i, h]:
                s0, v = acc.pop((i, h))
                assert s0 > 0
                finish(2 * i + h, v)


class _Jobs:
    def __init__(self, side=()):
        self.res = []
        self.side = list(side)

    def mm(self, lhs, wt, dot):
        acc = None
        for x, w in zip(lhs, wt):
            v = dot(x, w)
            self.res.append(v)
            acc = v if acc is None else v + acc
            rel = 4 * (len(self.res) % 4)
            while self.side and self.side[0][0] <= len(self.res):
                self.side.pop(0)[1](v[8 * rel:8 * rel + 8, :])
                rel = (rel + 2) % 16
        return acc


def _proj_step(h_scr, hs_scr, c_ref, cs_scr, wq_ref, wuk_ref, wuv_ref, q_scr, k_scr, v_scr, scale, shifts, side):
    wk, wvT, wq = [_PairWeights(w, n == 1, shifts[n]) for n, w in enumerate((wuk_ref, wuv_ref, wq_ref))]
    c_get = lambda f: _ldb(cs_scr, _C_SUMS[f]) if len(f) > 1 else c_ref[_tile(f[0][1]), _tile(f[0][2])]
    h_get = lambda f: _ldb(hs_scr, _H_SUMS[f]) if len(f) > 1 else _ldb(h_scr, f[0][1], f[0][2])

    def put(dst, w, mul=None):
        muls = [mul, _rows(w.inv if mul is None else w.inv * mul, T)]

        pend = {}

        def fn(u, v):
            v = (v if muls[u % 2] is None else v * muls[u % 2])
            if dst is v_scr:
                return _v_put(v_scr, pend, u // 2, u % 2, v)
            v = v.astype(BF16)
            dst[u] = v.T if mul is not None and u < QT else v
        return fn

    jobs = _Jobs(side)
    parts = dict(k=(_C_GROUPS, c_get, wk, False, put(k_scr, wk)), v=(_C_GROUPS, c_get, wvT, True, put(v_scr, wvT)),
                 q=(_H_GROUPS, h_get, wq, False, put(q_scr, wq, scale)))
    for name, i in zip(PORD[::2], PORD[1::2]):
        groups, get, w, transposed, fin = parts[name]
        _run_group(jobs, groups[int(i)], get, w, transposed, fin)
    assert not jobs.side


def _inner_group(rows, cols, pairs):
    xs, ys = dict.fromkeys(x for x, _ in pairs), dict.fromkeys(y for _, y in pairs)
    used = set(xs) | set(ys) | {(x[0], y[1]) for x, y in pairs} | {(y[0], x[1]) for x, y in pairs}
    prods = []
    for i, j in xs:
        mates = [y for x, y in pairs if x == (i, j)]
        prods.append((((1, i, 0),), ((1, 0, j), (-1, 1, j)), ((1, i, j),) + tuple((1, i2, j) for i2, _ in mates)))
        prods.append((((1, i, 0), (1, i, 1)), ((1, 1, j),), ((1, i, j),) + tuple((-1, i, j2) for _, j2 in mates)))
    for i2, j2 in ys:
        mates = [x for x, y in pairs if y == (i2, j2)]
        prods.append((((1, i2, 0), (1, i2, 1)), ((1, 0, j2),),
                      ((1, i2, j2),) + tuple((-1, i2, j) for _, j in mates)))
        prods.append((((1, i2, 1),), ((1, 0, j2), (-1, 1, j2)),
                      ((-1, i2, j2),) + tuple((-1, i, j2) for i, _ in mates)))
    prods += [(((1, i, h),), ((1, h, j),), ((1, i, j),))
              for i in rows for j in cols if (i, j) not in used for h in (0, 1)]
    for (i, j), (i2, j2) in pairs:
        lo, hi = min(j, j2), max(j, j2)
        prods.append((((1, i2, 0), (-1, i, 0)), ((1, 0, lo), (1, 0, hi)), ((1, i2, j),)))
        prods.append((((1, i, 0), (1, i2, 1)), ((1, 0, j2), (1, 1, j)), ((1, i, j2), (1, i2, j))))
        prods.append((((1, i, 1), (-1, i2, 1)), ((1, 1, lo), (1, 1, hi)), ((1, i, j2),)))
    return prods


def _o_jobs():
    prods = (_inner_group(range(10), range(5), _all_pairs(range(0, 10, 2), range(1, 10, 2)))
             + _inner_group(range(10, 16), range(5), _PAIRS65))
    need = lambda t: max(2 * (i // 2) + h for _, i, h in t[0])
    return [(need(t), t) for t in sorted(prods, key=need)]


_O_JOBS = _o_jobs()


def _job_order(nb):
    size = dict(a=2, b=1, d=2, o=2, e=0)
    qa, qe, qb = [], [], []
    for n in range(nb):
        a = UORD[n // 2]
        qa += [('a', n, (qi, c)) for c in range(2 * a + 2) for qi in range(2) if c <= 2 * a + qi]
        qe += [('e', n, (blk, sl)) for blk in range(a + 1) for sl in range(NSL)]
        qb += [('b', n, (m, blk)) for m in (3, 1, 2, 4, 0, 6, 5) for blk in range(a)]
        qb += [('d', n, j) for j in range(3)]
    qo = [('o', u, j) for j, (u, _) in enumerate(_O_JOBS)]
    qs = dict(a=qa, b=qb, o=qo, e=qe)
    done, order = {}, []
    now, next_e = 0, 0.0
    free = [0] * 4
    pops = []

    def emit(k):
        nonlocal now
        job = qs[k].pop(0)
        if k == 'e':
            _, nj, row = min(pops, key=lambda p: abs(p[0] - (next_e * 16 - LEADC)))
            job = job[:2] + (job[2] + (nj, row),)
        else:
            x = free.index(min(free))
            nj = sum(1 for j in order if j[0] != 'e')
            pops.extend((free[x] + 16 * g, nj, 16 * g) for g in range(4 * size[job[0]]))
            del pops[:-64]
            free[x] += 64 * size[job[0]]
        order.append(job)
        now += size[job[0]]
        if not qs[k] or qs[k][0][1] != job[1]:
            done[k, job[1]] = now

    def ok(k):
        if not qs[k]:
            return False
        n = qs[k][0][1]
        if k == 'a':
            return not qe or n - qe[0][1] < NBUF
        if k == 'e' and qb and n - qb[0][1] >= NBUF:
            return False
        prev, lat = dict(e=('a', LAT_A), b=('e', LAT_E), o=('b', LAT_B))[k]
        return (prev, n) in done and done[prev, n] + lat <= now

    def try_e():
        nonlocal next_e
        if ok('e') and next_e <= now:
            emit('e')
            next_e = max(next_e, now - 1) + DELTA
            return True

    while qa or qe or qb or qo:
        if try_e():
            continue
        cand = [k for k in 'abo' if ok(k)]
        if 'o' in cand and len(qo) <= RES and (qa or 'b' in cand):
            cand.remove('o')
        k = None
        if qe:
            ne = qe[0][1]
            n_e = (UORD[ne // 2] + 1) * NSL
            start = max(done.get(('e', ne - 1), 0), next_e - (n_e - sum(1 for j in qe if j[1] == ne)) * DELTA)
            dur = n_e * DELTA
            fa = 1 - sum(2 for j in qa if j[1] <= ne + 1) / (2 * (4 * UORD[min(ne + 1, nb - 1) // 2] + 3))
            fb = 1 - sum(size[j[0]] for j in qb if j[1] <= ne - 1) / (7 * UORD[max(ne - 1, 0) // 2] + 6)
            due = [((now - start + LAT_A * AX) / dur - fa, 'a'), ((now - start - LAT_E) / max(dur - LAT_E, 1) - fb, 'b')]
            best = max(due, key=lambda x: x[0] if x[1] in cand else -9)
            if best[1] in cand and best[0] > 0:
                k = best[1]
        if k is None:
            k = next((k for k in 'oab' if k in cand), None)
        if k:
            for _ in range(dict(a=GA, b=GB, o=GO)[k]):
                if ok(k):
                    emit(k)
                    try_e()
        else:
            now += 1
    return order


def _attention_step(q_scr, k_scr, v_scr, wo_ref, acc_scr, s_scr, f_scr, zero):
    causal = (jax.lax.broadcasted_iota(jnp.int32, (T, T), 0)
              <= jax.lax.broadcasted_iota(jnp.int32, (T, T), 1))
    mx, mfin, lsum, of, lhs = {}, {}, {}, {}, {}
    macc, dacc, left_b = {}, {}, {}
    res = []
    wo, terms = {}, {}
    left = {}
    for _, t in _O_JOBS:
        for _, i, j in t[2]:
            left[i, j] = left.get((i, j), 0) + 1
    H2 = T // 2

    def job_a(n, j):
        qi, c = j
        r, hd = 2 * UORD[n // 2] + qi, n % 2
        u = 2 * r + hd
        s = (_dot if u < QT else _dot_nt)(_ldb(k_scr, 2 * c + hd), _ldb(q_scr, u))
        res.append(s)
        if c == r:
            s = jnp.where(causal, s, -1e9 * LOG2E)
        s_scr[n % NBUF][zero + 2 * c + qi] = s
        pm = jnp.max(s.reshape(T // 8, 8, T), axis=0)
        mx[n, qi] = pm if (n, qi) not in mx else jnp.maximum(mx[n, qi], pm)

    def row_max(n, qi):
        m = jnp.broadcast_to(jnp.max(mx[n, qi], axis=0, keepdims=True), (8, T))
        if UORD[n // 2] == 0:
            return m
        nt = 2 * UORD[n // 2] + qi + 1
        cs = range(qi % BST, nt, BST)
        es = [jnp.exp2(s_scr[n % NBUF][2 * c + qi, 0:8, :] - m) for c in cs]
        while len(es) > 1:
            es = [es[i] + es[i + 1] if i + 1 < len(es) else es[i] for i in range(0, len(es), 2)]
        est = jnp.maximum(jnp.sum(es[0], axis=0, keepdims=True) * (16.0 * nt / len(cs)), 1.0)
        return m + jnp.log(est) * (0.5 * LOG2E)

    def job_e(n, j):
        blk, sl, nj, r0 = j
        rows = slice(sl * T // NSL, (sl + 1) * T // NSL)
        ms = []
        for qi in range(2):
            if (n, qi) not in mfin:
                mfin[n, qi] = row_max(n, qi)
            ms.append(_after(mfin[n, qi], res[nj][r0:r0 + 8, :]))

        def exps(qi, c):
            p = jnp.exp2(s_scr[n % NBUF][2 * c + qi, rows, :].reshape(-1, 8, T) - ms[qi][None])
            ls = jnp.sum(p, axis=0)
            lsum[n, qi] = ls if (n, qi) not in lsum else lsum[n, qi] + ls
            return p.reshape(-1, T)

        if blk == UORD[n // 2]:
            ops = [exps(qi, 2 * blk + kk) for qi, kk in ((0, 0), (1, 0), (1, 1))]
        else:
            ops = _b_ops(*[exps(qi, 2 * blk + kk) for kk in range(2) for qi in range(2)])
        for i, v in enumerate(ops):
            f_scr[n % NBUF][zero + blk, i, rows, :] = v.astype(BF16)

    def finish(n):
        left_b[n] = left_b.get(n, 7 * UORD[n // 2] + 3) - 1
        if left_b[n]:
            return
        d0, d1 = dacc[n, 0], dacc[n, 1]
        if UORD[n // 2]:
            c11, c12, c21, c22 = _strassen(lambda i: macc[n, i], lambda: (d0[:H2], d0[H2:]),
                                           lambda: (d1[:H2], d1[H2:]))
            d0, d1 = jnp.concatenate([c11, c21], axis=0), jnp.concatenate([c12, c22], axis=0)
        for qi, d in enumerate((d0, d1)):
            of[2 * (2 * (n // 2) + qi) + n % 2] = d * (1.0 / jnp.sum(lsum[n, qi], axis=0, keepdims=True))

    def job_b(n, j):
        m, blk = j
        v = _dot(_ldb(v_scr, n % 2, blk, m), _ldb(f_scr[n % NBUF], blk, m))
        res.append(v)
        macc[n, m] = v if (n, m) not in macc else v + macc[n, m]
        finish(n)

    def job_d(n, j):
        a, vu = UORD[n // 2], v_scr.bitcast(U32)
        i0, i1 = ((2, 7), (2, 7), (8, 3))[j]
        vt = pltpu.bitcast(jnp.concatenate([vu[n % 2, a, i0], vu[n % 2, a, i1]], axis=0), BF16)
        v = _dot(vt, _ldb(f_scr[n % NBUF], a, j))
        res.append(v)
        dacc[n, min(j, 1)] = v if (n, min(j, 1)) not in dacc else v + dacc[n, min(j, 1)]
        finish(n)

    def job_o(_, n):
        af, bf, outs = _O_JOBS[n][1]
        if af not in lhs:
            v = _form(af, lambda i, h: of[2 * i + h])
            lhs[af] = _tie(v.astype(BF16).T, v[0:8, :])
        if bf not in wo:
            wo[bf] = (wo_ref[_tile(bf[0][1]), _tile(bf[0][2])] if len(bf) == 1 else
                      _form(bf, lambda h, j: wo_ref[_tile(h), _tile(j)].astype(F32)).astype(BF16))
        v = _dot(lhs[af], wo[bf])
        res.append(v)
        for sign, i, j in outs:
            terms.setdefault((i, j), []).append((sign, v))
            if len(terms[i, j]) == left[i, j]:
                rows = _tile(2 * UORD[i // 2] + i % 2)
                tot = acc_scr[rows, _tile(j)]
                for sg, m in terms.pop((i, j)):
                    tot = tot + m if sg > 0 else tot - m
                acc_scr[rows, _tile(j)] = tot

    fns = dict(a=job_a, e=job_e, b=job_b, d=job_d, o=job_o)
    for kind, u, j in _job_order(q_scr.shape[0] // 2):
        fns[kind](u, j)


def _v_put(v_scr, pend, i, hd, v):
    pend[i, hd] = v
    if (i ^ 1, hd) in pend:
        lo, hi = pend.pop((i & ~1, hd)), pend.pop((i | 1, hd))
        H2 = T // 2
        a11, a12, a21, a22 = lo[:H2], hi[:H2], lo[H2:], hi[H2:]
        for m, x in enumerate(_a_ops(a11, a12, a21, a22) + [a21, a12]):
            v_scr[hd, i // 2, m] = x.astype(BF16)


def _kernel(x_hbm, c_hbm, wq_hbm, wuk_hbm, wuv_hbm, wo_hbm, w1_hbm, w2_hbm, w3_hbm, w4_hbm,
            cond_hbm, wmod_hbm, out_hbm,
            x_ref, c_ref, cond_ref, wma_ref, wmb_ref, w1_ref, w2_ref, w3_ref, w4_ref,
            wq_buf, wk_buf, wv_buf, wo_buf, out_buf, sem, wsem, osem,
            mod_scr, h_scr, cs_scr, hs_scr, w_scr, q_scr, k_scr, v_scr, acc_scr, xn_scr, xh_scr, a1_scr, t_scr,
            ws12, ws3, ws4, pq_buf, pk_buf, pv_buf, gap_scr, st_in, *rest):
    f_scr, s_scr = rest[:NBUF], rest[NBUF:]
    S, M = x_hbm.shape
    D = wq_hbm.shape[2]
    nattn = wo_hbm.shape[0]
    Fd = w4_hbm.shape[0]
    scale = float(D) ** -0.5 * LOG2E
    nb, nrb = S // T, S // RB
    km, kc = M // T, c_hbm.shape[1] // T
    NX = 4
    XR = S // NX
    CB = XR // T

    work, probe = (wk_buf, wv_buf, wq_buf), (pk_buf, pv_buf, pq_buf)

    def pcopies(g, bufs=work, s0=0):
        return [pltpu.make_async_copy(src.bitcast(U32).at[:, g, :], dst, wsem.at[s0 + j])
                for j, (src, dst) in enumerate(zip((wuk_hbm, wuv_hbm, wq_hbm), bufs))]

    def ocopy(g):
        return pltpu.make_async_copy(wo_hbm.at[g], wo_buf, wsem.at[3])

    def chunk_copy(src, dst, i, s0):
        rows = slice(i * XR, (i + 1) * XR)
        return pltpu.make_async_copy(src.at[rows, :], dst.at[rows, :], sem.at[s0 + i])

    cp_cond = pltpu.make_async_copy(cond_hbm, cond_ref, sem.at[0])
    cp_wma = pltpu.make_async_copy(wmod_hbm.at[:, 0:2 * M], wma_ref, sem.at[1])
    cp_late = [pltpu.make_async_copy(src, dst, sem.at[2 + j]) for j, (src, dst) in enumerate((
        (wmod_hbm.at[:, 2 * M:6 * M], wmb_ref), (w1_hbm, w1_ref), (w2_hbm, w2_ref),
        (w3_hbm, w3_ref), (w4_hbm, w4_ref)))]
    cp_x = [chunk_copy(x_hbm, x_ref, i, 7) for i in range(NX)]
    cp_c = [chunk_copy(c_hbm, c_ref, i, 7 + NX) for i in range(NX)]

    def silu_cond():
        cf = cond_ref[...].astype(F32)
        return jnp.broadcast_to((cf * jax.nn.sigmoid(cf)).astype(BF16), (8, M))

    cp_wk, cp_wv, cp_wq = pcopies(0)
    named = dict(k=cp_wk, v=cp_wv, q=cp_wq, o=ocopy(0), n=cp_cond, m=cp_wma)
    named.update(zip('abcd', cp_c))
    named.update(zip('wxyz', cp_x))
    started, arrived, did = set(), set(), set()
    vpend = {}

    def zero(r, carry):
        acc_scr[pl.ds(pl.multiple_of(r * T, T), T), :] = jnp.zeros((T, M), F32)
        return carry

    def x_rows(rows, dep):
        xf = x_ref[rows, :].astype(F32)
        if dep is None:
            return xf
        return jnp.concatenate([_after(xf[:, :T], _rows(dep, xf.shape[0])), xf[:, T:]], axis=1)

    def n_item(r, i):
        def fn(dep):
            rows = slice(r * T + i * LP, r * T + (i + 1) * LP)
            xn_scr[rows, :] = _ln(x_rows(rows, dep))
        return fn

    def h_item(r, i, normed):
        def fn(dep):
            rows = slice(i * LP, (i + 1) * LP)
            grows = slice(r * T + i * LP, r * T + (i + 1) * LP)
            sa = mod_scr[:, 0:M]
            if normed and dep is not None:
                sa = jnp.concatenate([_after(sa[:, _tile(j)], dep) for j in range(km)], axis=1)
            hf = ((xn_scr[grows, :] if normed else _ln(x_rows(grows, dep))) * _rows(mod_scr[:, M:2 * M], LP)
                  + _rows(sa, LP))
            for j in range(km):
                h_scr[r, j, rows, :] = hf[:, _tile(j)].astype(BF16)
            for f, n in _H_SUMS.items():
                if all(t[1] == r for t in f):
                    hs_scr[n, rows, :] = _form(f, lambda _, k: hf[:, _tile(k)]).astype(BF16)
            did.add(('h', r, i))
        return fn

    def release(jobs, span, items):
        if span and items:
            jobs.side += [(len(jobs.res) + 1 + i * span // len(items), fn) for i, fn in enumerate(items)]
            jobs.side.sort(key=lambda e: e[0])
        else:
            for fn in items:
                fn(None)

    def sum_items(n, group, index, dst, get, skip_rows):
        forms = [f for f in dict.fromkeys(t[0] for t in group)
                 if len(f) > 1 and not (skip_rows and len({t[1] for t in f}) == 1)]

        def item(f, rows):
            def fn(dep):
                def term(r, k):
                    v = get(r, k, rows).astype(F32)
                    return v if dep is None or (r, k) != f[0][1:] else _after(v, _rows(dep, v.shape[0]))
                dst[index[f], rows, :] = _form(f, term).astype(BF16)
            return fn

        return [item(f, slice(i, i + n)) for i in range(0, T, n) for f in forms]

    h_sums = lambda n, gi: sum_items(n, _H_GROUPS[gi], _H_SUMS, hs_scr,
                                     lambda r_, k, rows: h_scr[r_, k, rows, :], True)

    def stash(key, buf, j0, transpose=False):
        n = buf.shape[0] // T
        if key not in did:
            assert key in arrived
            did.add(key)
            w = _PairWeights(buf, transpose)
            for j in range(n):
                for hd in range(2):
                    w_scr[hd, j0 + j] = w(((1, j, hd),))[1]
        return lambda hd: [_ldb(w_scr, hd, j0 + j) for j in range(n)]

    def kv_tile(jobs, r):
        wk, wvT = stash('k', wk_buf, 0), stash('v', wv_buf, kc, True)
        ct = [c_ref[_tile(r), _tile(j)] for j in range(kc)]
        for hd in range(2):
            k_scr[2 * r + hd] = jobs.mm(ct, wk(hd), _dot).astype(BF16)
        for hd in range(2):
            _v_put(v_scr, vpend, r, hd, jobs.mm(wvT(hd), ct, _dot_nt))

    def q_tile(jobs, r):
        wq = stash('q', wq_buf, 2 * kc)
        ht = [_ldb(h_scr, r, j) for j in range(km)]
        for hd in range(2):
            v = (jobs.mm(ht, wq(hd), _dot) * scale).astype(BF16)
            q_scr[2 * r + hd] = v.T if 2 * r + hd < QT else v

    for blk in PROLOGUE.split(';'):
        waits, starts, acts = blk.split('|')
        for ch in waits.strip():
            assert ch in started and ch not in arrived
            arrived.add(ch)
            named[ch].wait()
        for ch in starts.strip():
            assert ch not in started
            started.add(ch)
            named[ch].start()
        jobs = _Jobs()
        for act in acts.split():
            if act == 'Z':
                jax.lax.fori_loop(0, nb, zero, 0)
                acc_scr[S:, :] = jnp.zeros((acc_scr.shape[0] - S, M), F32)
                x_ref[S:, :] = jnp.zeros((x_ref.shape[0] - S, M), BF16)
            elif act == 'L':
                did.add('L')
                for cp in cp_late:
                    cp.start()
            elif act == 'M':
                assert arrived >= set('nm')
                mod = _dot(silu_cond(), wma_ref[...])
                mod_scr[:, 0:M] = mod[:, 0:M]
                mod_scr[:, M:2 * M] = 1.0 + mod[:, M:2 * M]
                did.add('M')
            else:
                act, _, span = act.partition('@')
                span = int(span or 0)
                items = []
                for r in [int(ch, 16) for ch in act[1:]]:
                    did.add((act[0], r))
                    if act[0] == 'K':
                        assert 'abcd'[r // CB] in arrived
                        kv_tile(jobs, r)
                    elif act[0] == 'H':
                        assert 'wxyz'[r // CB] in arrived and 'M' in did
                        items += [h_item(r, i, ('N', r) in did) for i in range(T // LP)]
                    elif act[0] == 'N':
                        assert 'wxyz'[r // CB] in arrived
                        items += [n_item(r, i) for i in range(T // LP)]
                    elif act[0] == 'Q':
                        assert all(('h', r, i) in did for i in range(T // LP))
                        q_tile(jobs, r)
                    elif act[0] == 'C':
                        assert all('abcd'[t[1] // CB] in arrived for p_ in _C_GROUPS[r] for t in p_[0])
                        items += sum_items(
                            32, _C_GROUPS[r], _C_SUMS, cs_scr,
                            lambda r_, k, rows: c_ref[r_ * T + rows.start:r_ * T + rows.stop, _tile(k)], False)
                    else:
                        assert act[0] == 'S' and all(('h', t[1], T // LP - 1) in did for p_ in _H_GROUPS[r] for t in p_[0])
                        items += h_sums(32 if span else 16, r)
                release(jobs, span, items)
        assert not jobs.side
    assert arrived == set(named) and all((k_, r) in did for k_ in 'KHQ' for r in range(nb))
    assert all((k_, r) in did for k_ in 'CS' for r in range(2)) and 'L' in did

    FH = ws3.shape[0] * T
    assert nattn - 1 >= FH // 64

    slices = ((w1_hbm, 32, 2 * T, 0), (w2_hbm, 32, 2 * T, 64), (w4_hbm, 64, FH, 128), (w3_hbm, T, FH, 256))
    slice_of = lambda g, n, half: jnp.minimum(g, half // n - 1)

    def prep_in(g):
        return [pltpu.make_async_copy(
            w.at[pl.ds(pl.multiple_of(slice_of(g, n, half) * n + x * half, n), n), 0:4 * T],
            st_in.at[r0 + x * n:r0 + (x + 1) * n, :], wsem.at[7]) for w, n, half, r0 in slices for x in range(2)]

    def mixer_prep(g):
        def blocks(r0, n, half, c0, c1, dep):
            get = lambda x, c: st_in[r0 + x * half:r0 + x * half + n, _tile(c)].astype(F32)
            return [_after(get(0, c0), _rows(dep, n)), get(0, c1), get(1, c0), _after(get(1, c1), _rows(dep, n))]

        def rows_item(dst, per, half, r0, c, o, n=16):
            def fn(dep):
                rows = pl.ds(pl.multiple_of(slice_of(g, per, half) * (per // 2), per // 2) + o // 2, n // 2)
                for i, v in enumerate(_b_ops(*blocks(r0 + o, n, per, c, c + 2, dep))):
                    dst[i, c, rows, :] = _pk(v.astype(BF16))
            return fn

        def w3_item(k, i):
            def fn(dep):
                b11, b21, b12, b22 = blocks(slices[3][3], T, T, k, k + 2, dep)
                ws3[slice_of(g, T, FH), i, k] = _pk(_b_ops(b11, b12, b21, b22)[i].astype(BF16).T)
            return fn

        return ([rows_item(dst, *sl[1:], c, o) for dst, sl in zip((ws12.at[0], ws12.at[1], ws4), slices)
                 for c in range(2) for o in range(0, sl[1], 16)]
                + [w3_item(k, i) for k in range(2) for i in range(7)])

    def next_copies(g):
        return pcopies(jnp.minimum(g + 1, nattn - 1)) + pcopies(jnp.minimum(g + 2, nattn - 1), probe, 4)

    for cp in next_copies(0) + prep_in(0):
        cp.start()

    def attn_body(g, carry):
        copies = next_copies(g)

        _attention_step(q_scr, k_scr, v_scr, wo_buf, acc_scr, s_scr, f_scr, jnp.minimum(g, 0))
        for cp in copies:
            cp.wait()
        pltpu.make_async_copy(st_in, st_in, wsem.at[7]).wait()

        @pl.when(g == 0)
        def _():
            for fn in _gap_items(work, gap_scr):
                fn(None)

        @pl.when(g + 1 < nattn)
        def _():
            ocopy(g + 1).start()
            side = mixer_prep(g) + _gap_items(probe, gap_scr)
            side = [(SD0 + i * SDS + (SDJ if i >= SDN else 0), fn) for i, fn in enumerate(side)]
            _proj_step(h_scr, hs_scr, c_ref, cs_scr, wq_buf, wk_buf, wv_buf, q_scr, k_scr, v_scr, scale,
                       gap_scr, side)
            for cp in next_copies(g + 1) + prep_in(g + 1):
                cp.start()
            ocopy(g + 1).wait()

        return carry

    jax.lax.fori_loop(0, nattn, attn_body, 0)

    for cp in cp_late:
        cp.wait()
    mod = _dot(silu_cond(), wmb_ref[...])
    mod_scr[:, 2 * M:4 * M] = mod[:, 0:2 * M]
    mod_scr[:, 4 * M:5 * M] = 1.0 + mod[:, 2 * M:3 * M]
    mod_scr[:, 5 * M:6 * M] = mod[:, 3 * M:4 * M]
    ftiles = [(f, min(f + T, Fd)) for f in range(0, Fd, T)]
    OFF = x_ref.shape[0] - S
    CAR = t_scr.shape[0] - RB

    def p1(r0, l0, n, dep=None):
        ga = mod_scr[:, 2 * M:3 * M]
        if dep is not None:
            ga = jnp.concatenate([_after(ga[:, 0:T], dep), ga[:, T:]], axis=1)
        rows = pl.ds(r0, n)
        x1 = x_ref[rows, :].astype(F32) + _rows(ga, n) * acc_scr[rows, :]
        xh_scr[0, l0:l0 + n, :] = x1
        hb = _ln(x1) * _rows(mod_scr[:, 4 * M:5 * M], n) + _rows(mod_scr[:, 3 * M:4 * M], n)
        xh_scr[1, l0:l0 + n, :] = hb
        return _ln(hb)

    HT = T // 2

    def p1_store(r0, c, dep=None):
        v = p1(r0 + c * PC, OFF + c * PC, PC, dep)
        a1_scr[c * PC:(c + 1) * PC, :] = v
        return jnp.max(v[:, M - T:].reshape(PC // 8, 8, T), axis=0)

    t_scr[RB:RB + CAR - OFF, :] = jnp.zeros((CAR - OFF, M), F32)
    t_scr[RB + CAR - OFF:RB + CAR, :] = _gelu(_dot(p1(0, 0, OFF).astype(BF16), w1_ref[...]))
    for c in range(RB // PC):
        p1_store(OFF, c)

    def out_copy(i):
        rows = pl.ds(i * T if isinstance(i, int) else pl.multiple_of(i * T, T), T)
        return pltpu.make_async_copy(out_buf.at[rows, :], out_hbm.at[rows, :], osem.at[i])

    def b_body(r, carry):
        gb = _rows(mod_scr[:, 5 * M:6 * M], T)
        r0 = pl.multiple_of(r * RB, RB)
        n0 = pl.multiple_of(jnp.minimum(r0 + RB, S - RB) + OFF, OFF)
        nh = RB // T
        now = [0]
        due = []
        pace = []

        def p1_item(c):
            return lambda dep: due.append((now[0] + PD, p1_store(n0, c, dep)))

        pace += [(P0 + i * PSTEP, p1_item(i)) for i in range(RB // PC)]
        wt = lambda ref, f0, f1, n: ref[f0:f1, _tile(n)]

        def mm(lhs, wts, dot=_dot):
            acc = None
            for x, w in zip(lhs, wts):
                if due and due[0][0] <= now[0]:
                    w = _tie(w, due.pop(0)[1])
                v = dot(x, w)
                now[0] += x.shape[0] // HT
                acc = v if acc is None else v + acc
                if pace and pace[0][0] <= now[0]:
                    pace.pop(0)[1](v[0:8, :])
            return acc

        def split_ops(lo, hi):
            return [v.astype(BF16) for v in _a_ops(lo[:HT], hi[:HT], lo[HT:], hi[HT:])]

        def two_tiles(aops, wsel, rest):
            def col(w):
                v = mm(rest[0], w, rest[3])
                return v[:HT], v[HT:]

            c11, c12, c21, c22 = _strassen(
                lambda i: mm([a[i] for a in aops], [wsel(i, k) for k in range(len(aops))]),
                lambda: col(rest[1]), lambda: col(rest[2]))
            return jnp.concatenate([c11, c21], axis=0), jnp.concatenate([c12, c22], axis=0)

        def square(full, aops, w_ref, ws_ref):
            out = {}
            for n in range(2):
                out[n], out[n + 2] = two_tiles(
                    aops, lambda i, k: _ld(ws_ref, i, n, slice(k * HT, (k + 1) * HT)),
                    (full[4:], [wt(w_ref, 4 * T, M, n)], [wt(w_ref, 4 * T, M, n + 2)], _dot))
            out[4] = mm(full, [wt(w_ref, j * T, (j + 1) * T, 4) for j in range(km)])
            return out

        t_scr[0:CAR, :] = t_scr[RB:RB + CAR, :]
        for hf in range(nh):
            a1 = [a1_scr[_tile(hf), _tile(j)] for j in range(km)]
            full = [v.astype(BF16) for v in a1]
            aops = [split_ops(a1[k], a1[2 + k]) for k in range(2)]
            for n, v in square(full, aops, w1_ref, ws12.at[0]).items():
                t = _gelu(v)
                if hf == nh - 1:
                    t = jnp.concatenate([t[:T - OFF], jnp.where(r < nrb - 1, t[T - OFF:], 0.0)], axis=0)
                t_scr[CAR + hf * T:CAR + (hf + 1) * T, _tile(n)] = t
        cq = M // 4
        shifts = (-1, 1, -2, 2)
        lane = jax.lax.broadcasted_iota(jnp.int32, (T, T), 1)
        y1, z, a3 = [], [], []
        for hf in range(nh):
            base = CAR - OFF + hf * T
            sh = []
            for j in range(km):
                g_lo, g_hi = (j * T) // cq, ((j + 1) * T - 1) // cq
                assert g_hi - g_lo <= 1
                v = t_scr[base + shifts[g_lo]:base + shifts[g_lo] + T, _tile(j)]
                if g_hi != g_lo:
                    v2 = t_scr[base + shifts[g_hi]:base + shifts[g_hi] + T, _tile(j)]
                    v = jnp.where(lane < g_hi * cq - j * T, v, v2)
                sh.append(v)
            hs = square([v.astype(BF16) for v in sh], [split_ops(sh[k], sh[2 + k]) for k in range(2)],
                        w2_ref, ws12.at[1])
            hs = jnp.concatenate([hs[n] for n in range(km)], axis=1)
            y1.append(hs + xh_scr[1, _tile(hf), :])
            z.append(xh_scr[0, _tile(hf), :] + gb * y1[hf])
            a3.append({})

            def ln_item(hf, c):
                def item(dep):
                    n = HT // NLN
                    for d in (0, HT):
                        v = y1[hf][d + c * n:d + (c + 1) * n]
                        if dep is not None:
                            v = jnp.concatenate([_after(v[:, :T], _rows(dep, n)), v[:, T:]], axis=1)
                        a3[hf][d + c * n] = _ln(v)
                return item

            ln_item(hf, 0)(None)
            pace += [(now[0] + LN0 + (c - 1) * LNS * (1 + hf), ln_item(hf, c)) for c in range(1, NLN)]
            pace.sort(key=lambda e: e[0])
        xh_scr[:, 0:OFF, :] = xh_scr[:, RB:RB + OFF, :]
        nf = FH // T
        h3, h3ops = [], []
        for hf in range(nh):
            assert len(a3[hf]) == 2 * NLN
            af = jnp.concatenate([a3[hf][key] for key in sorted(a3[hf])], axis=0)
            full = [af[:, _tile(j)].astype(BF16) for j in range(km)]
            aops = [split_ops(af[:, _tile(k)], af[:, _tile(2 + k)]) for k in range(2)]
            row, ops = {}, []
            narrow = None
            for n in range(nf):
                lo, hi = two_tiles(aops, lambda i, k: _ld(ws3, n, i, k),
                                   (full[4:], [wt(w3_ref, *ftiles[n], 4)],
                                    [wt(w3_ref, *ftiles[nf + n], 4)], _dot_nt))
                lo, hi = _gelu(lo), _gelu(hi)
                row[n], row[nf + n] = lo.astype(BF16), hi.astype(BF16)
                ops.append(split_ops(lo, hi))
                if n < km:
                    v = mm([wt(w3_ref, *ftiles[-1], n)], [full[n]], _dot_nt)
                    narrow = v if narrow is None else v + narrow
            row[2 * nf] = _gelu(mm(full, [wt(w3_ref, *ftiles[2 * nf], j) for j in range(km)],
                                   _dot_nt)).astype(BF16)
            fw = Fd - ftiles[-1][0]
            gT = jnp.concatenate([_gelu(narrow), jnp.zeros((T - fw, T), F32)], axis=0)
            row[2 * nf + 1] = _tie(gT.astype(BF16).T, gT[0:8, :])[:, :fw]
            h3.append([row[i] for i in range(len(ftiles))])
            h3ops.append(ops)
        for hf in range(nh):
            rows = pl.ds(pl.multiple_of(r0 + hf * T, T), T)

            def finish(n, v):
                out_buf[rows, _tile(n)] = (z[hf][:, _tile(n)] + gb[:, _tile(n)] * v).astype(out_buf.dtype)

            w4t = lambda n, f_: [wt(w4_ref, f0, f1, n) for f0, f1 in f_]
            finish(4, mm(h3[hf], w4t(4, ftiles)))
            for n in range(2):
                lo, hi = two_tiles(h3ops[hf], lambda i, k: _ld(ws4, i, n, slice(k * HT, (k + 1) * HT)),
                                   (h3[hf][2 * nf:], w4t(n, ftiles[2 * nf:]), w4t(n + 2, ftiles[2 * nf:]), _dot))
                finish(n, lo)
                finish(n + 2, hi)
            out_copy(r * nh + hf).start()
        assert not pace
        return carry

    jax.lax.fori_loop(0, nrb, b_body, 0)
    for i in range(nb):
        out_copy(i).wait()


@jax.jit
def pallas_adaLN_cond__compressed_kv_cla__mixer_s_mlp__prompt_kernel(
    A_x: jax.Array,
    A_c_kv: jax.Array,
    A_w_q: jax.Array,
    A_w_uk: jax.Array,
    A_w_uv: jax.Array,
    A_w_o: jax.Array,
    B_x: jax.Array,
    B_w1: jax.Array,
    B_w2: jax.Array,
    B_w3: jax.Array,
    B_w4: jax.Array,
    c: jax.Array,
    w_mod: jax.Array,
):
    _, S, M = A_x.shape
    Dc = A_c_kv.shape[2]
    H, D = A_w_q.shape[1], A_w_q.shape[2]
    Fd = B_w3.shape[1]
    assert D == T and A_c_kv.shape[1] == S and Dc == 4 * T and M == 5 * T and 13 * T < Fd < 14 * T and S == 16 * T
    vmem = pltpu.VMEM
    packed = lambda *lead: vmem(lead + (T // 2, T), U32)
    out = pl.pallas_call(
        _kernel,
        in_specs=[pl.BlockSpec(memory_space=pltpu.HBM)] * 12,
        out_specs=pl.BlockSpec(memory_space=pltpu.HBM),
        out_shape=jax.ShapeDtypeStruct((S, M), A_x.dtype),
        scratch_shapes=[
            vmem((S + 16, M), BF16),
            vmem((S, Dc), BF16),
            vmem((1, M), BF16),
            vmem((M, 2 * M), BF16),
            vmem((M, 4 * M), BF16),
            vmem((M, M), BF16),
            vmem((M, M), BF16),
            vmem((Fd, M), BF16),
            vmem((Fd, M), BF16),
            vmem((M, D), U32),
            vmem((Dc, D), U32),
            vmem((Dc, D), U32),
            vmem((2 * D, M), BF16),
            vmem((S, M), A_x.dtype),
            pltpu.SemaphoreType.DMA((15,)),
            pltpu.SemaphoreType.DMA((8,)),
            pltpu.SemaphoreType.DMA((S // T,)),
            vmem((8, 6 * M), F32),
            vmem((S // T, M // T, T, T), BF16),
            vmem((len(_C_SUMS), T, T), BF16),
            vmem((len(_H_SUMS), T, T), BF16),
            vmem((2, M // T + 2 * (Dc // T), T, T), BF16),
            vmem((2 * S // T, T, T), BF16),
            vmem((2 * S // T, T, T), BF16),
            vmem((2, S // T // 2, 9, T // 2, T), BF16),
            vmem((S + 16, M), F32),
            vmem((S, M), F32),
            vmem((2, RB + 16, M), F32),
            vmem((RB, M), F32),
            vmem((RB + 32, M), F32),
            vmem((2, 7, 2, T, T), U32),
            packed(6, 7, 2),
            vmem((7, 2, 3 * T, T), U32),
            vmem((M, D), U32),
            vmem((Dc, D), U32),
            vmem((Dc, D), U32),
            vmem((3, 8, T), jnp.int32),
            vmem((4 * T, 4 * T), BF16),
        ] + [vmem((8, 7, T, T), BF16)] * NBUF + [vmem((32, T, T), F32)] * NBUF,
        compiler_params=pltpu.CompilerParams(
            vmem_limit_bytes=100 * 1024 * 1024,
            disable_bounds_checks=True,
        ),
    )(
        A_x.reshape(S, M), A_c_kv.reshape(S, Dc),
        A_w_q, A_w_uk, A_w_uv,
        A_w_o.reshape(H // 2, 2 * D, M),
        B_w1, B_w2, B_w3.T, B_w4, c, w_mod,
    )
    return out.reshape(1, S, M)
```
